```python
import jax
import jax.numpy as jnp

def _softmax(x, axis=-1):
    return jax.nn.softmax(x, axis=axis)
def _gelu(x):
    return jax.nn.gelu(x, approximate=True)
def _silu(x):
    return jax.nn.silu(x)
def _sigmoid(x):
    return jax.nn.sigmoid(x)
def _layernorm(x, axis=-1, eps=1e-5):
    m = jnp.mean(x, axis=axis, keepdims=True)
    v = jnp.var(x, axis=axis, keepdims=True)
    return (x - m) / jnp.sqrt(v + eps)
def _scatter_add(tgt, idx, src, axis=0):
    return tgt.at[idx].add(src)
def _segment_sum(src, seg, n):
    return jax.ops.segment_sum(src, seg, n)
class _Rng:
    def __init__(self, key):
        self._k = key
    def _next(self):
        self._k, sub = jax.random.split(self._k)
        return sub
    def normal(self, shape):
        return jax.random.normal(self._next(), shape, dtype=jnp.bfloat16)
    def randint(self, lo, hi, shape):
        return jax.random.randint(self._next(), shape, lo, hi, dtype=jnp.int32)
    def uniform(self, shape, lo=0.0, hi=1.0):
        return jax.random.uniform(self._next(), shape, jnp.bfloat16, lo, hi)
    def permutation(self, n):
        return jax.random.permutation(self._next(), n)


kernel_name = 'concat_heads__sliding_local_dilated__compressed_kv_cla__prompt'

def setup_inputs():
    _rng = _Rng(jax.random.key(int.from_bytes(__import__("os").urandom(4), "little")))
    _w = (lambda a: (lambda t: t.astype(jnp.bfloat16) if jnp.issubdtype(t.dtype, jnp.floating) else t)(jnp.asarray(a)))
    def _A_setup():
        B, S, D = 1, 2048, 1024
        return {
            "x": _w((lambda *s: _rng.normal(s) * 0.05)(B, S, D)),
            "wqkv": _w((lambda *s: _rng.normal(s) * 0.05)(D, 3 * D)),
            "wo": _w((lambda *s: _rng.normal(s) * 0.05)(D, D)),
        }
    _A_in = _A_setup()

    def _B_setup():
        B, H, Sq, Sk, D, M = 1, 32, 2048, 2048, 128, 1024
        Dc = 4 * D
        return {
            "x": _w((lambda *s: _rng.normal(s) * 0.05)(B, Sq, M)),
            "c_kv": _w((lambda *s: _rng.normal(s) * 0.05)(B, Sk, Dc)),
            "w_q": _w((lambda *s: _rng.normal(s) * 0.05)(M, H, D) * (M ** -0.5)),
            "w_uk": _w((lambda *s: _rng.normal(s) * 0.05)(Dc, H, D) * (Dc ** -0.5)),
            "w_uv": _w((lambda *s: _rng.normal(s) * 0.05)(Dc, H, D) * (Dc ** -0.5)),
            "w_o": _w((lambda *s: _rng.normal(s) * 0.05)(H, D, M) * ((H * D) ** -0.5)),
        }
    _B_in = _B_setup()

    return {
        "A_x": _A_in["x"],
        "A_wqkv": _A_in["wqkv"],
        "A_wo": _A_in["wo"],
        "B_x": _B_in["x"],
        "B_c_kv": _B_in["c_kv"],
        "B_w_q": _B_in["w_q"],
        "B_w_uk": _B_in["w_uk"],
        "B_w_uv": _B_in["w_uv"],
        "B_w_o": _B_in["w_o"],
    }

def reference(A_x, A_wqkv, A_wo, B_x, B_c_kv, B_w_q, B_w_uk, B_w_uv, B_w_o):
    def _A_ref(x, wqkv, wo):
        B, S, D = x.shape
        H = 32; Dh = D // H
        W, dil = 8, 2
        qkv = (lambda x, *d: x.transpose(*d))((x @ wqkv).reshape(B, S, 3, H, Dh), 2, 0, 3, 1, 4)
        q, k, v = qkv[0], qkv[1], qkv[2]
        scale = Dh ** -0.5
        pos = jnp.arange(S)
        off = jnp.arange(W) * dil
        idx = pos[:, None] - off[None, :]
        mask = idx >= 0
        idx_c = jnp.where(mask, idx, 0).reshape(-1)
        kg = k[:, :, idx_c, :].reshape(B, H, S, W, Dh)
        vg = v[:, :, idx_c, :].reshape(B, H, S, W, Dh)
        logits = jnp.einsum("bhsd,bhswd->bhsw", q, kg) * scale
        logits = jnp.where(mask[None, None, :, :], logits, -1e9)
        attn = _softmax(logits, axis=-1)
        o = jnp.einsum("bhsw,bhswd->bhsd", attn, vg)
        return (lambda x, *d: x.transpose(*d))(o, 0, 2, 1, 3).reshape(B, S, D) @ wo

    def _B_ref(x, c_kv, w_q, w_uk, w_uv, w_o):
        B, Sq, M = x.shape[0], x.shape[1], x.shape[2]
        Sk = c_kv.shape[1]
        H, D = w_q.shape[1], w_q.shape[2]
        q = jnp.einsum("bqm,mhd->bhqd", x, w_q)
        k = jnp.einsum("bkc,chd->bhkd", c_kv, w_uk)
        v = jnp.einsum("bkc,chd->bhkd", c_kv, w_uv)
        scores = jnp.einsum("bhqd,bhkd->bhqk", q, k) * (D ** -0.5)
        off = Sk - Sq
        qi = jnp.arange(Sq)[:, None]
        kj = jnp.arange(Sk)[None, :]
        cmask = kj <= (qi + off)
        scores = jnp.where(cmask[None, None], scores, -1e9)
        p = _softmax(scores, axis=-1)
        ctx = jnp.einsum("bhqk,bhkd->bhqd", p, v)
        return jnp.einsum("bhqd,hdm->bqm", ctx, w_o)

    a = _A_ref(A_x, A_wqkv, A_wo)
    b = _B_ref(B_x, B_c_kv, B_w_q, B_w_uk, B_w_uv, B_w_o)
    return jnp.concatenate([a, b], axis=-1)
```

```python
import functools
import math

import jax
import jax.numpy as jnp
import jax.experimental.pallas as pl
import jax.experimental.pallas.tpu as pltpu

bf16 = jnp.bfloat16
f32 = jnp.float32
u32 = jnp.uint32

NEG = -1e9
LOG2E = math.log2(math.e)
NT = (((1,), (1,)), ((), ()))

S = 2048
DM = 1024
HA, DH, WIN, DIL = 32, 32, 8, 2
TA = 128
NA = S // TA
HALO = 16
RC = 32
PC = 512
SCALE_A = DH ** -0.5 * LOG2E
HB, DB, DC = 32, 128, 512
TQ = 256
NQ = S // TQ
RT = TQ // 128
SCALE_B = DB ** -0.5 * LOG2E
TO = 256


def _pk(x):
    return pltpu.bitcast(x, u32)


def _upk(x):
    return pltpu.bitcast(x, bf16)


def _prep_wt(w_ref, t, wt_ref):
    for mc in range(DM // 128):
        blk = w_ref[mc * 128:(mc + 1) * 128, t * DM:(t + 1) * DM]
        y = blk.T.reshape(HA, DH, 128)
        y = jnp.swapaxes(y, 0, 1).reshape(DM, 128)
        wt_ref[t * 512:(t + 1) * 512, mc * 128:(mc + 1) * 128] = _pk(y)


def _prep_wo(wo_ref, wop_ref):
    for nc in range(DM // 128):
        y = wo_ref[:, nc * 128:(nc + 1) * 128].reshape(HA, DH, 128)
        y = jnp.swapaxes(y, 0, 1).reshape(DM, 128)
        wop_ref[:, nc * 128:(nc + 1) * 128] = _pk(y)


def _a_proj_piece(x_ref, wt_ref, r0, n, nxt):
    x = x_ref[pl.ds(r0, TA), :]
    w = _upk(wt_ref[n * PC // 2:(n + 1) * PC // 2, :])
    y = lax_dot_nt(x, w)
    for j in range(PC // 128):
        col = n * PC + j * 128
        t, g = col // DM, (col % DM) // 128
        blk = y[:, j * 128:(j + 1) * 128]
        if t == 0:
            nxt[0][g, :, :] = blk * SCALE_A
        else:
            nxt[t][g, HALO:HALO + TA, :] = blk


def lax_dot_nt(a, b):
    return jax.lax.dot_general(a, b, NT, preferred_element_type=f32)


def _a_attn_chunk(bufs, r0, c, o_ref):
    qv, kv, vv = bufs
    a = c * RC
    pos = r0 + a + jax.lax.broadcasted_iota(jnp.int32, (RC, 128), 0)
    q = [qv[g, a:a + RC, :] for g in range(8)]
    s = []
    for w in range(WIN):
        o = HALO + a - DIL * w
        acc = q[0] * kv[0, o:o + RC, :]
        for g in range(1, 8):
            acc = acc + q[g] * kv[g, o:o + RC, :]
        acc = acc + pltpu.roll(acc, 64, 1)
        acc = acc + pltpu.roll(acc, 32, 1)
        if w > 0:
            acc = jnp.where(pos >= DIL * w, acc, NEG)
        s.append(acc)
    m = s[0]
    for w in range(1, WIN):
        m = jnp.maximum(m, s[w])
    e = [jnp.exp2(s[w] - m) for w in range(WIN)]
    l = e[0]
    for w in range(1, WIN):
        l = l + e[w]
    inv = 1.0 / l
    cols = []
    for g in range(8):
        acc = e[0] * vv[g, HALO + a:HALO + a + RC, :]
        for w in range(1, WIN):
            o = HALO + a - DIL * w
            acc = acc + e[w] * vv[g, o:o + RC, :]
        cols.append(acc * inv)
    o_ref[a // 2:(a + RC) // 2, :] = _pk(jnp.concatenate(cols, axis=1).astype(bf16))


def _a_out_piece(o_ref, wop_ref, stage_ref, r0, n):
    y = jnp.dot(_upk(o_ref[...]), _upk(wop_ref[:, n * PC:(n + 1) * PC]),
                preferred_element_type=f32)
    stage_ref[pl.ds(r0, TA), n * PC:(n + 1) * PC] = y.astype(bf16)


def _a_stage(x_ref, wt_ref, wop_ref, stage_ref, out_copy, bufs, obuf,
             i, par, do_proj, do_attn, do_out, extra=()):
    cur, nxt = bufs[par], bufs[1 - par]
    if do_proj and do_attn:
        for t in (1, 2):
            nxt[t][:, 0:HALO, :] = cur[t][:, TA:TA + HALO, :]
    if do_attn:
        for c in range(TA // RC):
            _a_attn_chunk(cur, i * TA, c, obuf[par])
    for f in extra:
        f()
    if do_proj:
        rn = (i + 1) * TA
        if not isinstance(rn, int):
            rn = pl.multiple_of(rn, TA)
        for n in range(3 * DM // PC):
            _a_proj_piece(x_ref, wt_ref, rn, n, nxt)
    if do_out:
        rp = (i - 1) * TA
        if not isinstance(rp, int):
            rp = pl.multiple_of(rp, TA)
        for n in range(DM // PC):
            _a_out_piece(obuf[1 - par], wop_ref, stage_ref, rp, n)
        out_copy(i - 1).start()


def _b_deint_q(wq_raw, wq_d, mc):
    y = jnp.swapaxes(wq_raw[mc * 128:(mc + 1) * 128], 0, 1)
    wq_d[:, mc * 64:(mc + 1) * 64, :] = _pk(y)


def _b_deint_kv(w_raw, wkv_d, mc, half):
    y = jnp.swapaxes(w_raw[mc * 128:(mc + 1) * 128], 0, 1)
    wkv_d[:, mc * 64:(mc + 1) * 64, half * DB:(half + 1) * DB] = _pk(y)


def _b_retile(src, dst, r0, n):
    dst[r0 // 2:(r0 + n) // 2, :] = _pk(src[r0:r0 + n, :])


def _b_qk(i, q_s, k_s):
    base = i * TQ
    q = _upk(q_s[base // 2:(base + TQ) // 2, :])
    s0 = lax_dot_nt(q, _upk(k_s[0:(base + 128) // 2, :]))
    sd = [lax_dot_nt(q[t * 128:], _upk(k_s[(base + t * 128) // 2:(base + (t + 1) * 128) // 2, :]))
          for t in range(1, RT)]
    return s0, sd


def _b_softmax_pv(i, s0, sd, v_s, ctx_h):
    base = i * TQ
    row = jax.lax.broadcasted_iota(jnp.int32, (128, 128), 0)
    col = jax.lax.broadcasted_iota(jnp.int32, (128, 128), 1)
    tri = col <= row
    ps, ls = [], []
    for r in range(RT):
        parts = [s0[r * 128:(r + 1) * 128]]
        parts += [sd[t - 1][(r - t) * 128:(r - t + 1) * 128] for t in range(1, r + 1)]
        sr = jnp.concatenate(parts, axis=1) if len(parts) > 1 else parts[0]
        lr = base + (r + 1) * 128
        dg = jnp.where(tri, sr[:, lr - 128:], NEG)
        sr = jnp.concatenate([sr[:, :lr - 128], dg], axis=1) if lr > 128 else dg
        m = jnp.max(sr, axis=1, keepdims=True)
        p = jnp.exp2(sr - m)
        ls.append(jnp.sum(p, axis=1, keepdims=True))
        ps.append(p)
    p0 = jnp.concatenate([p[:, :base + 128] for p in ps], axis=0)
    o = jnp.dot(p0.astype(bf16), _upk(v_s[0:(base + 128) // 2, :]), preferred_element_type=f32)
    os_ = [o[r * 128:(r + 1) * 128] for r in range(RT)]
    for t in range(1, RT):
        lo, hi = base + t * 128, base + (t + 1) * 128
        pt = [ps[r][:, lo:hi] for r in range(t, RT)]
        pt = jnp.concatenate(pt, axis=0) if len(pt) > 1 else pt[0]
        ot = jnp.dot(pt.astype(bf16), _upk(v_s[lo // 2:hi // 2, :]), preferred_element_type=f32)
        for r in range(t, RT):
            os_[r] = os_[r] + ot[(r - t) * 128:(r - t + 1) * 128]
    for r in range(RT):
        lo = base + r * 128
        ctx_h[lo // 2:(lo + 128) // 2, :] = _pk((os_[r] * (1.0 / ls[r])).astype(bf16))


def _b_head(h, xb_p, ckv_p, wq_d, wkv_d, q_s, k_s, v_s, ctx):
    q = jnp.dot(_upk(xb_p[...]), _upk(wq_d[h]), preferred_element_type=f32) * SCALE_B
    q_s[...] = _pk(q.astype(bf16))
    kv = jnp.dot(_upk(ckv_p[...]), _upk(wkv_d[h]), preferred_element_type=f32)
    k_s[...] = _pk(kv[:, :DB].astype(bf16))
    v_s[...] = _pk(kv[:, DB:].astype(bf16))
    ctx_h = ctx.at[h]
    order = list(range(NQ))[::-1]
    nx = _b_qk(order[0], q_s, k_s)
    for n, i in enumerate(order):
        cu = nx
        if n + 1 < NQ:
            nx = _b_qk(order[n + 1], q_s, k_s)
        _b_softmax_pv(i, cu[0], cu[1], v_s, ctx_h)


def _kernel(xa_hbm, wqkv_hbm, woa_hbm, xb_hbm, ckv_hbm, wq_hbm, wuk_hbm, wuv_hbm, wob_hbm,
            out_hbm,
            xa, wqkv, woa, wt, wop, q0, k0, v0, q1, k1, v1, ob0, ob1, stage,
            xb, ckv, wq, wuk, wuv, wob, xb_p, ckv_p, wq_d, wkv_d, q_s, k_s, v_s, ctx,
            sem_in, sem_a, sem_b):
    def in_copy(idx, src, dst):
        return pltpu.make_async_copy(src, dst, sem_in.at[idx])

    c_w = [in_copy(t, wqkv_hbm.at[:, t * DM:(t + 1) * DM], wqkv.at[:, t * DM:(t + 1) * DM])
           for t in range(3)]
    c_xa = in_copy(3, xa_hbm, xa)
    c_woa = in_copy(4, woa_hbm, woa)
    c_wq = in_copy(5, wq_hbm, wq)
    c_wuk = in_copy(6, wuk_hbm, wuk)
    c_wuv = in_copy(7, wuv_hbm, wuv)
    c_ckv = in_copy(8, ckv_hbm, ckv)
    c_xb = in_copy(9, xb_hbm, xb)
    c_wob = in_copy(10, wob_hbm, wob)

    def a_out_copy(i):
        r = i * TA if isinstance(i, int) else pl.multiple_of(i * TA, TA)
        return pltpu.make_async_copy(stage.at[pl.ds(r, TA), :],
                                     out_hbm.at[pl.ds(r, TA), 0:DM], sem_a.at[i])

    def b_out_copy(i):
        r = i * TO if isinstance(i, int) else pl.multiple_of(i * TO, TO)
        return pltpu.make_async_copy(stage.at[pl.ds(r, TO), :],
                                     out_hbm.at[pl.ds(r, TO), DM:2 * DM], sem_b.at[i])

    for c in c_w:
        c.start()
    c_xa.start()
    c_woa.start()

    bufs = [(q0, k0, v0), (q1, k1, v1)]
    obuf = [ob0, ob1]
    k0[:, 0:HALO, :] = jnp.zeros((8, HALO, 128), f32)
    v0[:, 0:HALO, :] = jnp.zeros((8, HALO, 128), f32)
    for t in range(3):
        c_w[t].wait()
        if t == 0:
            for c in (c_wq, c_wuk, c_wuv, c_ckv, c_xb, c_wob):
                c.start()
        _prep_wt(wqkv, t, wt)
    c_xa.wait()
    c_woa.wait()
    st = functools.partial(_a_stage, xa, wt, wop, stage, a_out_copy, bufs, obuf)
    st(-1, 1, True, False, False, extra=[functools.partial(_prep_wo, woa, wop)])
    st(0, 0, True, True, False)

    def a_body(j, carry):
        st(2 * j + 1, 1, True, True, True)
        st(2 * j + 2, 0, True, True, True)
        return carry

    jax.lax.fori_loop(0, (NA - 2) // 2, a_body, 0)

    for c in (c_wq, c_wuk, c_wuv, c_ckv, c_xb):
        c.wait()
    extra = [functools.partial(_b_deint_q, wq, wq_d, mc) for mc in range(DM // 128)]
    extra += [functools.partial(_b_deint_kv, wuk, wkv_d, mc, 0) for mc in range(DC // 128)]
    extra += [functools.partial(_b_deint_kv, wuv, wkv_d, mc, 1) for mc in range(DC // 128)]
    extra += [functools.partial(_b_retile, xb, xb_p, r, 256) for r in range(0, S, 256)]
    extra += [functools.partial(_b_retile, ckv, ckv_p, r, 256) for r in range(0, S, 256)]
    st(NA - 1, 1, False, True, True, extra=extra)
    st(NA, 0, False, False, True)

    def b_body(h, carry):
        _b_head(h, xb_p, ckv_p, wq_d, wkv_d, q_s, k_s, v_s, ctx)
        return carry

    jax.lax.fori_loop(0, HB, b_body, 0)

    c_wob.wait()
    for i in range(NA):
        a_out_copy(i).wait()

    def o_body(i, carry):
        r2 = pl.multiple_of(i * (TO // 2), TO // 2)
        lhs = jnp.concatenate(
            [_upk(ctx[h, pl.ds(r2, TO // 2), :]) for h in range(HB)], axis=1)
        y = jnp.dot(lhs, wob[...], preferred_element_type=f32)
        stage[pl.ds(pl.multiple_of(i * TO, TO), TO), :] = y.astype(bf16)
        b_out_copy(i).start()
        return carry

    jax.lax.fori_loop(0, S // TO, o_body, 0)
    for i in range(S // TO):
        b_out_copy(i).wait()


@jax.jit
def pallas_concat_heads__sliding_local_dilated__compressed_kv_cla__prompt_kernel(
    A_x: jax.Array,
    A_wqkv: jax.Array,
    A_wo: jax.Array,
    B_x: jax.Array,
    B_c_kv: jax.Array,
    B_w_q: jax.Array,
    B_w_uk: jax.Array,
    B_w_uv: jax.Array,
    B_w_o: jax.Array,
):
    V = pltpu.VMEM
    slab = lambda n: V((8, n, 128), f32)
    scratch = [
        V((S, DM), bf16),
        V((DM, 3 * DM), bf16),
        V((DM, DM), bf16),
        V((3 * DM // 2, DM), u32),
        V((DM // 2, DM), u32),
        slab(TA), slab(TA + HALO), slab(TA + HALO),
        slab(TA), slab(TA + HALO), slab(TA + HALO),
        V((TA // 2, DM), u32), V((TA // 2, DM), u32),
        V((S, DM), bf16),
        V((S, DM), bf16),
        V((S, DC), bf16),
        V((DM, HB, DB), bf16),
        V((DC, HB, DB), bf16),
        V((DC, HB, DB), bf16),
        V((HB * DB, DM), bf16),
        V((S // 2, DM), u32),
        V((S // 2, DC), u32),
        V((HB, DM // 2, DB), u32),
        V((HB, DC // 2, 2 * DB), u32),
        V((S // 2, DB), u32), V((S // 2, DB), u32), V((S // 2, DB), u32),
        V((HB, S // 2, DB), u32),
        pltpu.SemaphoreType.DMA((11,)),
        pltpu.SemaphoreType.DMA((NA,)),
        pltpu.SemaphoreType.DMA((S // TO,)),
    ]
    any_spec = pl.BlockSpec(memory_space=pl.ANY)
    out = pl.pallas_call(
        _kernel,
        out_shape=jax.ShapeDtypeStruct((S, 2 * DM), bf16),
        in_specs=[any_spec] * 9,
        out_specs=any_spec,
        scratch_shapes=scratch,
        compiler_params=pltpu.CompilerParams(vmem_limit_bytes=120 * 1024 * 1024),
    )(
        A_x.reshape(S, DM), A_wqkv, A_wo,
        B_x.reshape(S, DM), B_c_kv.reshape(S, DC), B_w_q, B_w_uk, B_w_uv,
        B_w_o.reshape(HB * DB, DM),
    )
    return out.reshape(1, S, 2 * DM)
```

```python
import functools
import math

import jax
import jax.numpy as jnp
import jax.experimental.pallas as pl
import jax.experimental.pallas.tpu as pltpu

bf16 = jnp.bfloat16
f32 = jnp.float32
u32 = jnp.uint32

NEG = -1e9
LOG2E = math.log2(math.e)
NT = (((1,), (1,)), ((), ()))

S = 2048
DM = 1024
HA, DH, WIN, DIL = 32, 32, 8, 2
TA = 128
NA = S // TA
HALO = 16
RC = 32
PC = 512
SCALE_A = DH ** -0.5 * LOG2E
HB, DB, DC = 32, 128, 512
TQ = 256
NQ = S // TQ
RT = TQ // 128
SCALE_B = DB ** -0.5 * LOG2E
TO = 256


def _pk(x):
    return pltpu.bitcast(x, u32)


def _upk(x):
    return pltpu.bitcast(x, bf16)


def _recip(l):
    return pl.reciprocal(l, approx=False, full_range=False)


def _prep_wt(w_ref, t, wt_ref):
    for mc in range(DM // 128):
        blk = w_ref[mc * 128:(mc + 1) * 128, t * DM:(t + 1) * DM]
        y = blk.T.reshape(HA, DH, 128)
        y = jnp.swapaxes(y, 0, 1).reshape(DM, 128)
        wt_ref[t * 512:(t + 1) * 512, mc * 128:(mc + 1) * 128] = _pk(y)


def _prep_wo(wo_ref, wop_ref):
    for nc in range(DM // 128):
        y = wo_ref[:, nc * 128:(nc + 1) * 128].reshape(HA, DH, 128)
        y = jnp.swapaxes(y, 0, 1).reshape(DM, 128)
        wop_ref[:, nc * 128:(nc + 1) * 128] = _pk(y)


def _tie(w, z):
    if z is None:
        return w
    top = jnp.concatenate([w[0:8, 0:128] | z, w[0:8, 128:]], axis=1)
    return jnp.concatenate([top, w[8:]], axis=0)


def _token(o, zero):
    o = o.reshape(-1, o.shape[-1])
    acc = None
    for r in range(0, o.shape[0], 8):
        for c in range(0, o.shape[1], 128):
            v = o[r:r + 8, c:c + 128]
            acc = v if acc is None else acc | v
    return acc & zero


def _a_proj_piece(x_ref, wt_ref, r0, n, nxt, z=None):
    x = x_ref[pl.ds(r0, TA), :]
    w = _upk(_tie(wt_ref[n * PC // 2:(n + 1) * PC // 2, :], z))
    y = lax_dot_nt(x, w)
    for j in range(PC // 128):
        col = n * PC + j * 128
        t, g = col // DM, (col % DM) // 128
        blk = y[:, j * 128:(j + 1) * 128]
        if t == 0:
            nxt[0][g, :, :] = blk * SCALE_A
        else:
            nxt[t][g, HALO:HALO + TA, :] = blk


def lax_dot_nt(a, b):
    return jax.lax.dot_general(a, b, NT, preferred_element_type=f32)


def _a_attn_chunk(bufs, r0, c, o_ref):
    qv, kv, vv = bufs
    a = c * RC
    pos = r0 + a + jax.lax.broadcasted_iota(jnp.int32, (RC, 128), 0)
    q = [qv[g, a:a + RC, :] for g in range(8)]
    s = []
    for w in range(WIN):
        o = HALO + a - DIL * w
        acc = q[0] * kv[0, o:o + RC, :]
        for g in range(1, 8):
            acc = acc + q[g] * kv[g, o:o + RC, :]
        acc = acc + pltpu.roll(acc, 64, 1)
        acc = acc + pltpu.roll(acc, 32, 1)
        if w > 0:
            acc = jnp.where(pos >= DIL * w, acc, NEG)
        s.append(acc)
    m = s[0]
    for w in range(1, WIN):
        m = jnp.maximum(m, s[w])
    e = [jnp.exp2(s[w] - m) for w in range(WIN)]
    l = e[0]
    for w in range(1, WIN):
        l = l + e[w]
    inv = _recip(l)
    cols = []
    for g in range(8):
        acc = e[0] * vv[g, HALO + a:HALO + a + RC, :]
        for w in range(1, WIN):
            o = HALO + a - DIL * w
            acc = acc + e[w] * vv[g, o:o + RC, :]
        cols.append(acc * inv)
    o_ref[a // 2:(a + RC) // 2, :] = _pk(jnp.concatenate(cols, axis=1).astype(bf16))


def _a_out_piece(o_ref, wop_ref, stage_ref, r0, n, z=None):
    y = jnp.dot(_upk(o_ref[...]), _upk(_tie(wop_ref[:, n * PC:(n + 1) * PC], z)),
                preferred_element_type=f32)
    stage_ref[pl.ds(r0, TA), n * PC:(n + 1) * PC] = y.astype(bf16)


def _a_halo(cur, nxt, t):
    nxt[t][:, 0:HALO, :] = cur[t][:, TA:TA + HALO, :]


def _a_proj_third(x_ref, wt_ref, blk, t, dst):
    rn = blk * TA
    if not isinstance(rn, int):
        rn = pl.multiple_of(rn, TA)
    for n in range(t * DM // PC, (t + 1) * DM // PC):
        _a_proj_piece(x_ref, wt_ref, rn, n, dst)


def _a_attn(bufs, obuf, i, par):
    for c in range(TA // RC):
        _a_attn_chunk(bufs[par], i * TA, c, obuf[par])


def _a_out(wop_ref, stage_ref, out_copy, obuf, i, par):
    rp = i * TA
    if not isinstance(rp, int):
        rp = pl.multiple_of(rp, TA)
    for n in range(DM // PC):
        _a_out_piece(obuf[par], wop_ref, stage_ref, rp, n)
    out_copy(i).start()


def _a_stage(x_ref, wt_ref, wop_ref, stage_ref, out_copy, bufs, obuf,
             i, par, do_proj, side=()):
    if do_proj:
        for t in (1, 2):
            _a_halo(bufs[par], bufs[1 - par], t)
    _a_attn(bufs, obuf, i, par)
    mm = []
    if do_proj:
        rn = (i + 1) * TA
        if not isinstance(rn, int):
            rn = pl.multiple_of(rn, TA)
        mm += [functools.partial(_a_proj_piece, x_ref, wt_ref, rn, n, bufs[1 - par])
               for n in range(3 * DM // PC)]
    rp = (i - 1) * TA
    if not isinstance(rp, int):
        rp = pl.multiple_of(rp, TA)
    mm += [functools.partial(_a_out_piece, obuf[1 - par], wop_ref, stage_ref, rp, n)
           for n in range(DM // PC)]
    for f in side:
        f()
    for f in mm:
        f()
    out_copy(i - 1).start()


PQ = DM // 2 + 1
PK = DC // 2 + 1


def _head_block(h):
    return (h % 2) * (HB // 2) + h // 2


def _b_deint(raw, dst, pitch, r0, p0):
    span = (HB - 1) * pitch + 64
    view = dst.at[pl.ds(p0, span), :]
    x = pltpu.bitcast(raw[pl.ds(r0, 128)], u32).reshape(64, 2, HB // 2, DB)
    a, b = x[:, 0], x[:, 1]
    lo = (a & u32(0xFFFF)) | (b << 16)
    hi = (a >> 16) | (b & u32(0xFFFF0000))
    for p in range(64):
        for c, v in ((0, lo), (1, hi)):
            for half in range(2):
                blk = c * (HB // 2) + half * 8
                view[pl.ds(blk * pitch + p, 8, stride=pitch), :] = v[p, half * 8:(half + 1) * 8, :]


def _mult(x, n):
    return x if isinstance(x, int) else pl.multiple_of(x, n)


def _b_deint_q(wq_raw, wq_d, j):
    _b_deint(wq_raw, wq_d, PQ, _mult(j * 128, 128), _mult(j * 64, 64))


def _b_deint_kv(wukv_raw, wkv_d, j):
    _b_deint(wukv_raw, wkv_d.at[j // 4], PK, _mult(j * 128, 128), _mult((j % 4) * 64, 64))


def _b_qk(i, q_s, k_s):
    base = i * TQ
    q = _upk(q_s[base // 2:(base + TQ) // 2, :])
    s0 = lax_dot_nt(q, _upk(k_s[0:(base + 128) // 2, :]))
    sd = [lax_dot_nt(q[t * 128:], _upk(k_s[(base + t * 128) // 2:(base + (t + 1) * 128) // 2, :]))
          for t in range(1, RT)]
    return s0, sd


def _b_softmax_pv(i, s0, sd, v_s, ctx_h):
    base = i * TQ
    row = jax.lax.broadcasted_iota(jnp.int32, (128, 128), 0)
    col = jax.lax.broadcasted_iota(jnp.int32, (128, 128), 1)
    tri = col <= row
    ps, ls = [], []
    for r in range(RT):
        parts = [s0[r * 128:(r + 1) * 128]]
        parts += [sd[t - 1][(r - t) * 128:(r - t + 1) * 128] for t in range(1, r + 1)]
        sr = jnp.concatenate(parts, axis=1) if len(parts) > 1 else parts[0]
        lr = base + (r + 1) * 128
        dg = jnp.where(tri, sr[:, lr - 128:], NEG)
        sr = jnp.concatenate([sr[:, :lr - 128], dg], axis=1) if lr > 128 else dg
        m = jnp.max(sr, axis=1, keepdims=True)
        p = jnp.exp2(sr - m)
        ls.append(jnp.sum(p, axis=1, keepdims=True))
        ps.append(p)
    p0 = jnp.concatenate([p[:, :base + 128] for p in ps], axis=0)
    o = jnp.dot(p0.astype(bf16), _upk(v_s[0:(base + 128) // 2, :]), preferred_element_type=f32)
    os_ = [o[r * 128:(r + 1) * 128] for r in range(RT)]
    for t in range(1, RT):
        lo, hi = base + t * 128, base + (t + 1) * 128
        pt = [ps[r][:, lo:hi] for r in range(t, RT)]
        pt = jnp.concatenate(pt, axis=0) if len(pt) > 1 else pt[0]
        ot = jnp.dot(pt.astype(bf16), _upk(v_s[lo // 2:hi // 2, :]), preferred_element_type=f32)
        for r in range(t, RT):
            os_[r] = os_[r] + ot[(r - t) * 128:(r - t + 1) * 128]
    for r in range(RT):
        lo = base + r * 128
        ctx_h[lo // 2:(lo + 128) // 2, :] = _pk((os_[r] * _recip(ls[r])).astype(bf16))


def _b_head(h, xb, ckv, wq_d, wkv_d, q_s, k_s, v_s, ctx):
    blk = _head_block(h)
    wq = _upk(wq_d[pl.ds(blk * PQ, DM // 2), :])
    q = jnp.dot(xb[...], wq, preferred_element_type=f32) * SCALE_B
    q_s[...] = _pk(q.astype(bf16))
    wkv = jnp.concatenate([_upk(wkv_d[t, pl.ds(blk * PK, DC // 2), :]) for t in range(2)], axis=1)
    kv = jnp.dot(ckv[...], wkv, preferred_element_type=f32)
    k_s[...] = _pk(kv[:, :DB].astype(bf16))
    v_s[...] = _pk(kv[:, DB:].astype(bf16))
    ctx_h = ctx.at[h]
    order = list(range(NQ))[::-1]
    nx = _b_qk(order[0], q_s, k_s)
    for n, i in enumerate(order):
        cu = nx
        if n + 1 < NQ:
            nx = _b_qk(order[n + 1], q_s, k_s)
        _b_softmax_pv(i, cu[0], cu[1], v_s, ctx_h)


XC = 256
NU = 8
SEM_XA, SEM_WQ, SEM_WUKV, NSEM_IN = 7, 15, 23, 31


def _kernel(xa_hbm, wqkv_hbm, woa_hbm, xb_hbm, ckv_hbm, wq_hbm, wuk_hbm, wuv_hbm, wob_hbm,
            out_hbm,
            xa, wqkv, woa, wt, wop, q0, k0, v0, q1, k1, v1, ob0, ob1, stage,
            xb, ckv, wq, wukv, wob, wq_d, wkv_d, q_s, k_s, v_s, ctx,
            sem_in, sem_a, sem_b):
    def in_copy(idx, src, dst):
        return pltpu.make_async_copy(src, dst, sem_in.at[idx])

    def rows(j, n):
        return pl.ds(j * n if isinstance(j, int) else pl.multiple_of(j * n, n), n)

    c_w = [in_copy(t, wqkv_hbm.at[:, t * DM:(t + 1) * DM], wqkv.at[:, t * DM:(t + 1) * DM])
           for t in range(3)]
    c_woa = in_copy(3, woa_hbm, woa)
    c_ckv = in_copy(4, ckv_hbm, ckv)
    c_xb = in_copy(5, xb_hbm, xb)
    c_wob = in_copy(6, wob_hbm, wob)

    def c_xa(j):
        return pltpu.make_async_copy(xa_hbm.at[rows(j, XC)], xa.at[rows(j, XC)], sem_in.at[SEM_XA + j])

    def c_wq(j):
        return pltpu.make_async_copy(wq_hbm.at[rows(j, 128)], wq.at[rows(j, 128)], sem_in.at[SEM_WQ + j])

    def c_wukv_start(j):
        src = wuk_hbm.at[rows(j, 128)] if j < 4 else wuv_hbm.at[rows(j - 4, 128)]
        pltpu.make_async_copy(src, wukv.at[rows(j, 128)], sem_in.at[SEM_WUKV + j]).start()

    def c_wukv_wait(j):
        dst = wukv.at[rows(j, 128)]
        pltpu.make_async_copy(dst, dst, sem_in.at[SEM_WUKV + j]).wait()

    def a_out_copy(i):
        return pltpu.make_async_copy(stage.at[rows(i, TA), :],
                                     out_hbm.at[rows(i, TA), 0:DM], sem_a.at[i])

    def b_out_copy(i):
        return pltpu.make_async_copy(stage.at[rows(i, TO), :],
                                     out_hbm.at[rows(i, TO), DM:2 * DM], sem_b.at[i])

    c_w[0].start()
    c_xa(0).start()
    c_w[1].start()
    c_w[2].start()
    c_woa.start()
    for j in range(NU):
        if j + 1 < S // XC:
            c_xa(j + 1).start()
        c_wq(j).start()
        c_wukv_start(j)
    c_ckv.start()
    c_xb.start()
    c_wob.start()

    bufs = [(q0, k0, v0), (q1, k1, v1)]
    obuf = [ob0, ob1]
    k0[:, 0:HALO, :] = jnp.zeros((8, HALO, 128), f32)
    v0[:, 0:HALO, :] = jnp.zeros((8, HALO, 128), f32)
    proj = functools.partial(_a_proj_third, xa, wt)
    c_w[0].wait()
    _prep_wt(wqkv, 0, wt)
    c_xa(0).wait()
    proj(0, 0, bufs[0])
    c_w[1].wait()
    proj(1, 0, bufs[1])
    _prep_wt(wqkv, 1, wt)
    proj(0, 1, bufs[0])
    c_w[2].wait()
    proj(1, 1, bufs[1])
    _prep_wt(wqkv, 2, wt)
    proj(0, 2, bufs[0])
    c_woa.wait()
    for t in (1, 2):
        _a_halo(bufs[0], bufs[1], t)
    _a_attn(bufs, obuf, 0, 0)
    _prep_wo(woa, wop)
    proj(1, 2, bufs[1])

    st = functools.partial(_a_stage, xa, wt, wop, stage, a_out_copy, bufs, obuf)

    def a_body(j, carry):
        c_xa(j + 1).wait()
        c_wq(j).wait()
        c_wukv_wait(j)
        st(2 * j + 1, 1, True, side=[functools.partial(_b_deint_q, wq, wq_d, j)])
        st(2 * j + 2, 0, True, side=[functools.partial(_b_deint_kv, wukv, wkv_d, j)])
        return carry

    jax.lax.fori_loop(0, (NA - 2) // 2, a_body, 0)

    c_wq(NU - 1).wait()
    c_wukv_wait(NU - 1)
    st(NA - 1, 1, False, side=[functools.partial(_b_deint_q, wq, wq_d, NU - 1),
                               functools.partial(_b_deint_kv, wukv, wkv_d, NU - 1)])
    _a_out(wop, stage, a_out_copy, obuf, NA - 1, 1)
    c_ckv.wait()
    c_xb.wait()

    def b_body(h, carry):
        _b_head(h, xb, ckv, wq_d, wkv_d, q_s, k_s, v_s, ctx)
        return carry

    jax.lax.fori_loop(0, HB, b_body, 0)

    c_wob.wait()
    for i in range(NA):
        a_out_copy(i).wait()

    def o_body(i, carry):
        r2 = pl.multiple_of(i * (TO // 2), TO // 2)
        lhs = jnp.concatenate(
            [_upk(ctx[h, pl.ds(r2, TO // 2), :]) for h in range(HB)], axis=1)
        y = jnp.dot(lhs, wob[...], preferred_element_type=f32)
        stage[pl.ds(pl.multiple_of(i * TO, TO), TO), :] = y.astype(bf16)
        b_out_copy(i).start()
        return carry

    jax.lax.fori_loop(0, S // TO, o_body, 0)
    for i in range(S // TO):
        b_out_copy(i).wait()


@jax.jit
def pallas_concat_heads__sliding_local_dilated__compressed_kv_cla__prompt_kernel(
    A_x: jax.Array,
    A_wqkv: jax.Array,
    A_wo: jax.Array,
    B_x: jax.Array,
    B_c_kv: jax.Array,
    B_w_q: jax.Array,
    B_w_uk: jax.Array,
    B_w_uv: jax.Array,
    B_w_o: jax.Array,
):
    V = pltpu.VMEM
    slab = lambda n: V((8, n, 128), f32)
    scratch = [
        V((S, DM), bf16),
        V((DM, 3 * DM), bf16),
        V((DM, DM), bf16),
        V((3 * DM // 2, DM), u32),
        V((DM // 2, DM), u32),
        slab(TA), slab(TA + HALO), slab(TA + HALO),
        slab(TA), slab(TA + HALO), slab(TA + HALO),
        V((TA // 2, DM), u32), V((TA // 2, DM), u32),
        V((S, DM), bf16),
        V((S, DM), bf16),
        V((S, DC), bf16),
        V((DM, HB, DB), bf16),
        V((2 * DC, HB, DB), bf16),
        V((HB * DB, DM), bf16),
        V((HB * PQ, DB), u32),
        V((2, HB * PK, DB), u32),
        V((S // 2, DB), u32), V((S // 2, DB), u32), V((S // 2, DB), u32),
        V((HB, S // 2, DB), u32),
        pltpu.SemaphoreType.DMA((NSEM_IN,)),
        pltpu.SemaphoreType.DMA((NA,)),
        pltpu.SemaphoreType.DMA((S // TO,)),
    ]
    any_spec = pl.BlockSpec(memory_space=pl.ANY)
    out = pl.pallas_call(
        _kernel,
        out_shape=jax.ShapeDtypeStruct((S, 2 * DM), bf16),
        in_specs=[any_spec] * 9,
        out_specs=any_spec,
        scratch_shapes=scratch,
        compiler_params=pltpu.CompilerParams(vmem_limit_bytes=120 * 1024 * 1024),
    )(
        A_x.reshape(S, DM), A_wqkv, A_wo,
        B_x.reshape(S, DM), B_c_kv.reshape(S, DC), B_w_q, B_w_uk, B_w_uv,
        B_w_o.reshape(HB * DB, DM),
    )
    return out.reshape(1, S, 2 * DM)
```

```python
import functools
import math

import jax
import jax.numpy as jnp
import jax.experimental.pallas as pl
import jax.experimental.pallas.tpu as pltpu

bf16 = jnp.bfloat16
f32 = jnp.float32
u32 = jnp.uint32

NEG = -1e9
LOG2E = math.log2(math.e)
NT = (((1,), (1,)), ((), ()))

S = 2048
DM = 1024
HA, DH, WIN, DIL = 32, 32, 8, 2
TA = 128
NA = S // TA
HALO = 16
RC = 64
PC = 512
SCALE_A = DH ** -0.5 * LOG2E
HB, DB, DC = 32, 128, 512
TQ = 256
NQ = S // TQ
RT = TQ // 128
SCALE_B = DB ** -0.5 * LOG2E
TO = 256


def _pk(x):
    return pltpu.bitcast(x, u32)


def _upk(x):
    return pltpu.bitcast(x, bf16)


def _recip(l):
    return pl.reciprocal(l, approx=False, full_range=False)


def _prep_wt(w_ref, t, wt_ref, mcs=range(DM // 128)):
    for mc in mcs:
        blk = w_ref[mc * 128:(mc + 1) * 128, t * DM:(t + 1) * DM]
        y = blk.T.reshape(HA, DH, 128)
        y = jnp.swapaxes(y, 0, 1).reshape(DM, 128)
        wt_ref[t * 512:(t + 1) * 512, mc * 128:(mc + 1) * 128] = _pk(y)


def _prep_wo(wo_ref, wop_ref):
    for nc in range(DM // 128):
        y = wo_ref[:, nc * 128:(nc + 1) * 128].reshape(HA, DH, 128)
        y = jnp.swapaxes(y, 0, 1).reshape(DM, 128)
        wop_ref[:, nc * 128:(nc + 1) * 128] = _pk(y)


def _tie(w, z):
    if z is None:
        return w
    top = jnp.concatenate([w[0:8, 0:128] | z, w[0:8, 128:]], axis=1)
    return jnp.concatenate([top, w[8:]], axis=0)


def _token(o, zero):
    o = o.reshape(-1, o.shape[-1])
    acc = None
    for r in range(0, o.shape[0], 8):
        for c in range(0, o.shape[1], 128):
            v = o[r:r + 8, c:c + 128]
            acc = v if acc is None else acc | v
    return acc & zero


def _a_proj_piece(x_ref, wt_ref, r0, n, nxt, z=None):
    x = x_ref[pl.ds(r0, TA), :]
    w = _upk(_tie(wt_ref[n * PC // 2:(n + 1) * PC // 2, :], z))
    y = lax_dot_nt(x, w)
    for j in range(PC // 128):
        col = n * PC + j * 128
        t, g = col // DM, (col % DM) // 128
        blk = y[:, j * 128:(j + 1) * 128]
        if t == 0:
            nxt[0][g, :, :] = blk * SCALE_A
        else:
            nxt[t][g, HALO:HALO + TA, :] = blk


def lax_dot_nt(a, b):
    return jax.lax.dot_general(a, b, NT, preferred_element_type=f32)


def _or_zero(x, z):
    zt = z if x.shape[0] == 8 else jnp.concatenate([z] * (x.shape[0] // 8), axis=0)
    return pltpu.bitcast(pltpu.bitcast(x, u32) | zt, f32)


def _a_attn_chunk(bufs, r0, c, o_ref, zero=None, z=None):
    qv, kv, vv = bufs
    a = c * RC
    pos = r0 + a + jax.lax.broadcasted_iota(jnp.int32, (RC, 128), 0)
    q = [qv[g, a:a + RC, :] for g in range(8)]
    if z is not None:
        q = [_or_zero(x, z) for x in q]
    s = []
    for w in range(WIN):
        o = HALO + a - DIL * w
        acc = q[0] * kv[0, o:o + RC, :]
        for g in range(1, 8):
            acc = acc + q[g] * kv[g, o:o + RC, :]
        acc = acc + pltpu.roll(acc, 64, 1)
        acc = acc + pltpu.roll(acc, 32, 1)
        if w > 0:
            acc = jnp.where(pos >= DIL * w, acc, NEG)
        s.append(acc)
    m = s[0]
    for w in range(1, WIN):
        m = jnp.maximum(m, s[w])
    e = [jnp.exp2(s[w] - m) for w in range(WIN)]
    l = e[0]
    for w in range(1, WIN):
        l = l + e[w]
    inv = _recip(l)
    cols = []
    for g in range(8):
        acc = e[0] * vv[g, HALO + a:HALO + a + RC, :]
        for w in range(1, WIN):
            o = HALO + a - DIL * w
            acc = acc + e[w] * vv[g, o:o + RC, :]
        cols.append(acc * inv)
    o_ref[a // 2:(a + RC) // 2, :] = _pk(jnp.concatenate(cols, axis=1).astype(bf16))
    if zero is None:
        return None
    t = pltpu.bitcast(cols[0], u32)
    for g in range(1, 8):
        t = t | pltpu.bitcast(cols[g], u32)
    z = t[0:8]
    for r in range(8, RC, 8):
        z = z | t[r:r + 8]
    z = z & zero
    for _ in range(ATTN_DELAY):
        z = pltpu.roll(z, 1, 1)
    return z


ATTN_CHAIN = False
ATTN_DELAY = 0


def _a_out_piece(o_ref, wop_ref, stage_ref, r0, n, z=None):
    y = jnp.dot(_upk(o_ref[...]), _upk(_tie(wop_ref[:, n * PC:(n + 1) * PC], z)),
                preferred_element_type=f32)
    stage_ref[pl.ds(r0, TA), n * PC:(n + 1) * PC] = y.astype(bf16)


def _a_halo(cur, nxt, t):
    nxt[t][:, 0:HALO, :] = cur[t][:, TA:TA + HALO, :]


def _a_proj_third(x_ref, wt_ref, blk, t, dst):
    rn = blk * TA
    if not isinstance(rn, int):
        rn = pl.multiple_of(rn, TA)
    for n in range(t * DM // PC, (t + 1) * DM // PC):
        _a_proj_piece(x_ref, wt_ref, rn, n, dst)


def _a_attn(bufs, obuf, i, par, zero=None, z=None):
    if not ATTN_CHAIN:
        zero = None
    for c in range(TA // RC):
        z = _a_attn_chunk(bufs[par], i * TA, c, obuf[par], zero, z)
    return z


def _a_out(wop_ref, stage_ref, out_copy, obuf, i, par):
    rp = i * TA
    if not isinstance(rp, int):
        rp = pl.multiple_of(rp, TA)
    for n in range(DM // PC):
        _a_out_piece(obuf[par], wop_ref, stage_ref, rp, n)
    out_copy(i).start()


def _a_stage(x_ref, wt_ref, wop_ref, stage_ref, out_copy, bufs, obuf,
             i, par, do_proj, side=(), zero=None):
    if do_proj:
        for t in (1, 2):
            _a_halo(bufs[par], bufs[1 - par], t)
    _a_attn(bufs, obuf, i, par, zero)
    mm = []
    if do_proj:
        rn = (i + 1) * TA
        if not isinstance(rn, int):
            rn = pl.multiple_of(rn, TA)
        mm += [functools.partial(_a_proj_piece, x_ref, wt_ref, rn, n, bufs[1 - par])
               for n in range(3 * DM // PC)]
    rp = (i - 1) * TA
    if not isinstance(rp, int):
        rp = pl.multiple_of(rp, TA)
    mm += [functools.partial(_a_out_piece, obuf[1 - par], wop_ref, stage_ref, rp, n)
           for n in range(DM // PC)]
    for f in side:
        f()
    for f in mm:
        f()
    out_copy(i - 1).start()


PQ = DM // 2 + 1
PK = DC // 2 + 1


def _head_block(h):
    return (h % 2) * (HB // 2) + h // 2


def _b_deint(raw, dst, pitch, r0, p0, zero=None, z=None):
    span = (HB - 1) * pitch + 64
    view = dst.at[pl.ds(p0, span), :]
    src = raw.at[pl.ds(r0, 128)]
    for p in range(64):
        x = pltpu.bitcast(src[2 * p:2 * p + 2], u32)
        a, b = x[0], x[1]
        if z is not None:
            a = a | jnp.concatenate([z, z], axis=0)
        lo = (a & u32(0xFFFF)) | (b << 16)
        hi = (a >> 16) | (b & u32(0xFFFF0000))
        for c, v in ((0, lo), (1, hi)):
            for half in range(2):
                blk = c * (HB // 2) + half * 8
                view[pl.ds(blk * pitch + p, 8, stride=pitch), :] = v[half * 8:(half + 1) * 8, :]
        if zero is not None:
            t = lo | hi
            z = (t[0:8] | t[8:16]) & zero
            if DELAY_EVERY and p % DELAY_EVERY == DELAY_EVERY - 1:
                z = pltpu.roll(z, 1, 1)
    return z


DELAY_EVERY = 3


def _mult(x, n):
    return x if isinstance(x, int) else pl.multiple_of(x, n)


def _b_deint_q(wq_raw, wq_d, j, zero=None, z=None):
    return _b_deint(wq_raw, wq_d, PQ, _mult(j * 128, 128), _mult(j * 64, 64), zero, z)


def _b_deint_kv(wukv_raw, wkv_d, j, zero=None, z=None):
    return _b_deint(wukv_raw, wkv_d.at[j // 4], PK, _mult(j * 128, 128), _mult((j % 4) * 64, 64),
                    zero, z)


def _b_qk(i, q_s, k_s):
    base = i * TQ
    q = _upk(q_s[base // 2:(base + TQ) // 2, :])
    s0 = lax_dot_nt(q, _upk(k_s[0:(base + 128) // 2, :]))
    sd = [lax_dot_nt(q[t * 128:], _upk(k_s[(base + t * 128) // 2:(base + (t + 1) * 128) // 2, :]))
          for t in range(1, RT)]
    return s0, sd


def _b_softmax_pv(i, s0, sd, v_s, ctx_h):
    base = i * TQ
    row = jax.lax.broadcasted_iota(jnp.int32, (128, 128), 0)
    col = jax.lax.broadcasted_iota(jnp.int32, (128, 128), 1)
    tri = col <= row
    ps, ls = [], []
    for r in range(RT):
        parts = [s0[r * 128:(r + 1) * 128]]
        parts += [sd[t - 1][(r - t) * 128:(r - t + 1) * 128] for t in range(1, r + 1)]
        sr = jnp.concatenate(parts, axis=1) if len(parts) > 1 else parts[0]
        lr = base + (r + 1) * 128
        dg = jnp.where(tri, sr[:, lr - 128:], NEG)
        sr = jnp.concatenate([sr[:, :lr - 128], dg], axis=1) if lr > 128 else dg
        m = jnp.max(sr, axis=1, keepdims=True)
        p = jnp.exp2(sr - m)
        ls.append(jnp.sum(p, axis=1, keepdims=True))
        ps.append(p)
    p0 = jnp.concatenate([p[:, :base + 128] for p in ps], axis=0)
    o = jnp.dot(p0.astype(bf16), _upk(v_s[0:(base + 128) // 2, :]), preferred_element_type=f32)
    os_ = [o[r * 128:(r + 1) * 128] for r in range(RT)]
    for t in range(1, RT):
        lo, hi = base + t * 128, base + (t + 1) * 128
        pt = [ps[r][:, lo:hi] for r in range(t, RT)]
        pt = jnp.concatenate(pt, axis=0) if len(pt) > 1 else pt[0]
        ot = jnp.dot(pt.astype(bf16), _upk(v_s[lo // 2:hi // 2, :]), preferred_element_type=f32)
        for r in range(t, RT):
            os_[r] = os_[r] + ot[(r - t) * 128:(r - t + 1) * 128]
    for r in range(RT):
        lo = base + r * 128
        ctx_h[lo // 2:(lo + 128) // 2, :] = _pk((os_[r] * _recip(ls[r])).astype(bf16))


def _b_head(h, xb, ckv, wq_d, wkv_d, q_s, k_s, v_s, ctx):
    blk = _head_block(h)
    wq = _upk(wq_d[pl.ds(blk * PQ, DM // 2), :])
    q = jnp.dot(xb[...], wq, preferred_element_type=f32) * SCALE_B
    q_s[...] = _pk(q.astype(bf16))
    wkv = jnp.concatenate([_upk(wkv_d[t, pl.ds(blk * PK, DC // 2), :]) for t in range(2)], axis=1)
    kv = jnp.dot(ckv[...], wkv, preferred_element_type=f32)
    k_s[...] = _pk(kv[:, :DB].astype(bf16))
    v_s[...] = _pk(kv[:, DB:].astype(bf16))
    ctx_h = ctx.at[h]
    order = list(range(NQ))[::-1]
    nx = _b_qk(order[0], q_s, k_s)
    for n, i in enumerate(order):
        cu = nx
        if n + 1 < NQ:
            nx = _b_qk(order[n + 1], q_s, k_s)
        _b_softmax_pv(i, cu[0], cu[1], v_s, ctx_h)


XC = 256
NU = 8
WCH = (4, 2, 2)
SEM_W = (0, 4, 6)
SEM_WOA, SEM_CKV, SEM_XB, SEM_WOB, SEM_XA = 8, 9, 10, 11, 12
SEM_WQ = SEM_XA + S // XC
SEM_WUKV = SEM_WQ + NU
NSEM_IN = SEM_WUKV + NU


def _kernel(xa_hbm, wqkv_hbm, woa_hbm, xb_hbm, ckv_hbm, wq_hbm, wuk_hbm, wuv_hbm, wob_hbm,
            out_hbm,
            xa, wqkv, woa, wt, wop, q0, k0, v0, q1, k1, v1, ob0, ob1, stage,
            xb, ckv, wq, wukv, wob, wq_d, wkv_d, q_s, k_s, v_s, ctx,
            zero_s, sem_in, sem_a, sem_b):
    def in_copy(idx, src, dst):
        return pltpu.make_async_copy(src, dst, sem_in.at[idx])

    def rows(j, n):
        return pl.ds(j * n if isinstance(j, int) else pl.multiple_of(j * n, n), n)

    def c_w(t, c):
        r = rows(c, DM // WCH[t])
        cols = slice(t * DM, (t + 1) * DM)
        return in_copy(SEM_W[t] + c, wqkv_hbm.at[r, cols], wqkv.at[r, cols])

    def c_xa(j):
        return in_copy(SEM_XA + j, xa_hbm.at[rows(j, XC)], xa.at[rows(j, XC)])

    c_woa = in_copy(SEM_WOA, woa_hbm, woa)

    def c_wq(j):
        return in_copy(SEM_WQ + j, wq_hbm.at[rows(j, 128)], wq.at[rows(j, 128)])

    def c_wukv_start(j):
        src = wuk_hbm.at[rows(j, 128)] if j < 4 else wuv_hbm.at[rows(j - 4, 128)]
        in_copy(SEM_WUKV + j, src, wukv.at[rows(j, 128)]).start()

    def c_wukv_wait(j):
        dst = wukv.at[rows(j, 128)]
        in_copy(SEM_WUKV + j, dst, dst).wait()

    c_ckv = in_copy(SEM_CKV, ckv_hbm, ckv)
    c_xb = in_copy(SEM_XB, xb_hbm, xb)
    c_wob = in_copy(SEM_WOB, wob_hbm, wob)

    def a_out_copy(i):
        return pltpu.make_async_copy(stage.at[rows(i, TA), :],
                                     out_hbm.at[rows(i, TA), 0:DM], sem_a.at[i])

    def b_out_copy(i):
        return pltpu.make_async_copy(stage.at[rows(i, TO), :],
                                     out_hbm.at[rows(i, TO), DM:2 * DM], sem_b.at[i])

    for c in range(WCH[0]):
        c_w(0, c).start()
    c_xa(0).start()
    for t in (1, 2):
        for c in range(WCH[t]):
            c_w(t, c).start()
    c_woa.start()
    for j in range(NU):
        if j + 1 < S // XC:
            c_xa(j + 1).start()
        c_wq(j).start()
        c_wukv_start(j)
    for c in (c_ckv, c_xb, c_wob):
        c.start()
    zero_s[0] = jnp.uint32(0)

    bufs = [(q0, k0, v0), (q1, k1, v1)]
    obuf = [ob0, ob1]
    k0[:, 0:HALO, :] = jnp.zeros((8, HALO, 128), f32)
    v0[:, 0:HALO, :] = jnp.zeros((8, HALO, 128), f32)
    proj = functools.partial(_a_proj_third, xa, wt)
    for c in range(4):
        c_w(0, c).wait()
        _prep_wt(wqkv, 0, wt, range(2 * c, 2 * c + 2))
    c_xa(0).wait()
    proj(0, 0, bufs[0])
    c_w(1, 0).wait()
    proj(1, 0, bufs[1])
    _prep_wt(wqkv, 1, wt, range(0, 4))
    c_w(1, 1).wait()
    _prep_wt(wqkv, 1, wt, range(4, 8))
    proj(0, 1, bufs[0])
    c_w(2, 0).wait()
    proj(1, 1, bufs[1])
    _prep_wt(wqkv, 2, wt, range(0, 4))
    c_w(2, 1).wait()
    _prep_wt(wqkv, 2, wt, range(4, 8))
    proj(0, 2, bufs[0])
    for t in (1, 2):
        _a_halo(bufs[0], bufs[1], t)
    _a_attn(bufs, obuf, 0, 0)
    proj(1, 2, bufs[1])
    c_woa.wait()
    _prep_wo(woa, wop)

    st = functools.partial(_a_stage, xa, wt, wop, stage, a_out_copy, bufs, obuf)

    def a_body(j, carry):
        c_xa(j + 1).wait()
        c_wq(j).wait()
        c_wukv_wait(j)
        zero = jnp.full((8, 128), zero_s[0], u32)
        z = _b_deint_q(wq, wq_d, j, zero)
        _b_deint_kv(wukv, wkv_d, j, zero, z)
        st(2 * j + 1, 1, True, zero=zero)
        st(2 * j + 2, 0, True, zero=zero)
        return carry

    jax.lax.fori_loop(0, (NA - 2) // 2, a_body, 0)

    c_wq(NU - 1).wait()
    c_wukv_wait(NU - 1)
    st(NA - 1, 1, False, side=[functools.partial(_b_deint_q, wq, wq_d, NU - 1),
                               functools.partial(_b_deint_kv, wukv, wkv_d, NU - 1)])
    _a_out(wop, stage, a_out_copy, obuf, NA - 1, 1)
    c_ckv.wait()
    c_xb.wait()

    def b_body(h, carry):
        _b_head(h, xb, ckv, wq_d, wkv_d, q_s, k_s, v_s, ctx)
        return carry

    jax.lax.fori_loop(0, HB, b_body, 0)

    c_wob.wait()
    for i in range(NA):
        a_out_copy(i).wait()

    def o_body(i, carry):
        r2 = pl.multiple_of(i * (TO // 2), TO // 2)
        lhs = jnp.concatenate(
            [_upk(ctx[h, pl.ds(r2, TO // 2), :]) for h in range(HB)], axis=1)
        y = jnp.dot(lhs, wob[...], preferred_element_type=f32)
        stage[pl.ds(pl.multiple_of(i * TO, TO), TO), :] = y.astype(bf16)
        b_out_copy(i).start()
        return carry

    jax.lax.fori_loop(0, S // TO, o_body, 0)
    for i in range(S // TO):
        b_out_copy(i).wait()


@jax.jit
def pallas_concat_heads__sliding_local_dilated__compressed_kv_cla__prompt_kernel(
    A_x: jax.Array,
    A_wqkv: jax.Array,
    A_wo: jax.Array,
    B_x: jax.Array,
    B_c_kv: jax.Array,
    B_w_q: jax.Array,
    B_w_uk: jax.Array,
    B_w_uv: jax.Array,
    B_w_o: jax.Array,
):
    V = pltpu.VMEM
    slab = lambda n: V((8, n, 128), f32)
    scratch = [
        V((S, DM), bf16),
        V((DM, 3 * DM), bf16),
        V((DM, DM), bf16),
        V((3 * DM // 2, DM), u32),
        V((DM // 2, DM), u32),
        slab(TA), slab(TA + HALO), slab(TA + HALO),
        slab(TA), slab(TA + HALO), slab(TA + HALO),
        V((TA // 2, DM), u32), V((TA // 2, DM), u32),
        V((S, DM), bf16),
        V((S, DM), bf16),
        V((S, DC), bf16),
        V((DM, HB, DB), bf16),
        V((2 * DC, HB, DB), bf16),
        V((HB * DB, DM), bf16),
        V((HB * PQ, DB), u32),
        V((2, HB * PK, DB), u32),
        V((S // 2, DB), u32), V((S // 2, DB), u32), V((S // 2, DB), u32),
        V((HB, S // 2, DB), u32),
        pltpu.SMEM((1,), u32),
        pltpu.SemaphoreType.DMA((NSEM_IN,)),
        pltpu.SemaphoreType.DMA((NA,)),
        pltpu.SemaphoreType.DMA((S // TO,)),
    ]
    any_spec = pl.BlockSpec(memory_space=pl.ANY)
    out = pl.pallas_call(
        _kernel,
        out_shape=jax.ShapeDtypeStruct((S, 2 * DM), bf16),
        in_specs=[any_spec] * 9,
        out_specs=any_spec,
        scratch_shapes=scratch,
        compiler_params=pltpu.CompilerParams(vmem_limit_bytes=120 * 1024 * 1024),
    )(
        A_x.reshape(S, DM), A_wqkv, A_wo,
        B_x.reshape(S, DM), B_c_kv.reshape(S, DC), B_w_q, B_w_uk, B_w_uv,
        B_w_o.reshape(HB * DB, DM),
    )
    return out.reshape(1, S, 2 * DM)
```

```python
import functools
import math

import jax
import jax.numpy as jnp
import jax.experimental.pallas as pl
import jax.experimental.pallas.tpu as pltpu

bf16 = jnp.bfloat16
f32 = jnp.float32
u32 = jnp.uint32

NEG = -1e9
LOG2E = math.log2(math.e)
NT = (((1,), (1,)), ((), ()))

S = 2048
DM = 1024
HA, DH, WIN, DIL = 32, 32, 8, 2
TA = 128
NA = S // TA
HALO = 16
RC = 64
PC = 512
SCALE_A = DH ** -0.5 * LOG2E
HB, DB, DC = 32, 128, 512
TQ = 256
NQ = S // TQ
RT = TQ // 128
SCALE_B = DB ** -0.5 * LOG2E
TO = 256


def _pk(x):
    return pltpu.bitcast(x, u32)


def _upk(x):
    return pltpu.bitcast(x, bf16)


def _tree(xs, op):
    xs = list(xs)
    while len(xs) > 1:
        xs = [op(xs[k], xs[k + 1]) if k + 1 < len(xs) else xs[k] for k in range(0, len(xs), 2)]
    return xs[0]


def _dot_nt(a, b):
    return jax.lax.dot_general(a, b, NT, preferred_element_type=f32)


def _recip(l):
    return pl.reciprocal(l, approx=False, full_range=False)


PW = HA // 2 + 1
NW = DH * PW


def _repack_heads(u, dst, base):
    for hp in range(HA // 2):
        a = u[(2 * hp) * 16:(2 * hp + 1) * 16]
        b = u[(2 * hp + 1) * 16:(2 * hp + 2) * 16]
        lo = (a & u32(0xFFFF)) | (b << 16)
        hi = (a >> 16) | (b & u32(0xFFFF0000))
        for k, v in enumerate((lo[0:8], lo[8:16], hi[0:8], hi[8:16])):
            dst[pl.ds(base + k * 8 * PW + hp, 8, stride=PW), :] = v


def _load_slots(src, base, s0, s1):
    return jnp.concatenate([src[base + d * PW:base + d * PW + 16, :] for d in range(s0, s1)], axis=0)


def _prep_wt(w_ref, t, wt_ref, mcs=range(DM // 128)):
    for mc in mcs:
        blk = w_ref[mc * 128:(mc + 1) * 128, t * DM:(t + 1) * DM]
        _repack_heads(_pk(blk.T), wt_ref.at[mc], t * NW)


def _prep_wo(wo_ref, wop_ref):
    for nc in range(DM // 128):
        _repack_heads(_pk(wo_ref[:, nc * 128:(nc + 1) * 128]), wop_ref.at[nc], 0)


def _a_proj_piece(x_ref, wt_ref, r0, n, nxt):
    x = x_ref[pl.ds(r0, TA), :]
    t, s0 = (n * PC) // DM, ((n * PC) % DM) // HA
    w = jnp.concatenate([_load_slots(wt_ref.at[mc], t * NW, s0, s0 + PC // HA)
                         for mc in range(DM // 128)], axis=1)
    y = _dot_nt(x, _upk(w))
    for j in range(PC // 128):
        col = n * PC + j * 128
        t, g = col // DM, (col % DM) // 128
        blk = y[:, j * 128:(j + 1) * 128]
        if t == 0:
            nxt[0][g, :, :] = blk * SCALE_A
        else:
            nxt[t][g, HALO:HALO + TA, :] = blk


def _a_attn_chunk(bufs, r0, c, o_ref):
    qv, kv, vv = bufs
    a = c * RC
    pos = r0 + a + jax.lax.broadcasted_iota(jnp.int32, (RC, 128), 0)
    q = [qv[g, a:a + RC, :] for g in range(8)]
    s = []
    for w in range(WIN):
        o = HALO + a - DIL * w
        acc = q[0] * kv[0, o:o + RC, :]
        for g in range(1, 8):
            acc = acc + q[g] * kv[g, o:o + RC, :]
        acc = acc + pltpu.roll(acc, 64, 1)
        acc = acc + pltpu.roll(acc, 32, 1)
        if w > 0:
            acc = jnp.where(pos >= DIL * w, acc, NEG)
        s.append(acc)
    m = s[0]
    for w in range(1, WIN):
        m = jnp.maximum(m, s[w])
    e = [jnp.exp2(s[w] - m) for w in range(WIN)]
    l = e[0]
    for w in range(1, WIN):
        l = l + e[w]
    inv = _recip(l)
    cols = []
    for g in range(8):
        acc = e[0] * vv[g, HALO + a:HALO + a + RC, :]
        for w in range(1, WIN):
            o = HALO + a - DIL * w
            acc = acc + e[w] * vv[g, o:o + RC, :]
        cols.append(acc * inv)
    o_ref[a // 2:(a + RC) // 2, :] = _pk(jnp.concatenate(cols, axis=1).astype(bf16))


def _a_out_piece(o_ref, wop_ref, stage_ref, r0, n):
    w = jnp.concatenate([_load_slots(wop_ref.at[nc], 0, 0, DH)
                         for nc in range(n * PC // 128, (n + 1) * PC // 128)], axis=1)
    y = jnp.dot(_upk(o_ref[...]), _upk(w), preferred_element_type=f32)
    stage_ref[pl.ds(r0, TA), n * PC:(n + 1) * PC] = y.astype(bf16)


def _a_halo(cur, nxt, t):
    nxt[t][:, 0:HALO, :] = cur[t][:, TA:TA + HALO, :]


def _a_proj_third(x_ref, wt_ref, blk, t, dst):
    rn = blk * TA
    if not isinstance(rn, int):
        rn = pl.multiple_of(rn, TA)
    for n in range(t * DM // PC, (t + 1) * DM // PC):
        _a_proj_piece(x_ref, wt_ref, rn, n, dst)


def _a_attn(bufs, obuf, i, par):
    for c in range(TA // RC):
        _a_attn_chunk(bufs[par], i * TA, c, obuf[par])


def _a_out(wop_ref, stage_ref, out_copy, obuf, i, par):
    rp = i * TA
    if not isinstance(rp, int):
        rp = pl.multiple_of(rp, TA)
    for n in range(DM // PC):
        _a_out_piece(obuf[par], wop_ref, stage_ref, rp, n)
    out_copy(i).start()


def _a_stage(x_ref, wt_ref, wop_ref, stage_ref, out_copy, bufs, obuf,
             i, par, do_proj, side=()):
    if do_proj:
        for t in (1, 2):
            _a_halo(bufs[par], bufs[1 - par], t)
    _a_attn(bufs, obuf, i, par)
    mm = []
    if do_proj:
        rn = (i + 1) * TA
        if not isinstance(rn, int):
            rn = pl.multiple_of(rn, TA)
        mm += [functools.partial(_a_proj_piece, x_ref, wt_ref, rn, n, bufs[1 - par])
               for n in range(3 * DM // PC)]
    rp = (i - 1) * TA
    if not isinstance(rp, int):
        rp = pl.multiple_of(rp, TA)
    mm += [functools.partial(_a_out_piece, obuf[1 - par], wop_ref, stage_ref, rp, n)
           for n in range(DM // PC)]
    for f in side:
        f()
    for f in mm:
        f()
    out_copy(i - 1).start()


PQ = DM // 2 + 1
PK = DC // 2 + 1


def _head_block(h):
    return (h % 2) * (HB // 2) + h // 2


def _b_deint(raw, dst, pitch, r0, p0, zero=None, z=None, delay=None):
    span = (HB - 1) * pitch + 64
    view = dst.at[pl.ds(p0, span), :]
    src = raw.at[pl.ds(r0, 128)]
    for p in range(64):
        x = pltpu.bitcast(src[2 * p:2 * p + 2], u32)
        a, b = x[0], x[1]
        if z is not None:
            a = a | jnp.concatenate([z, z], axis=0)
        lo = (a & u32(0xFFFF)) | (b << 16)
        hi = (a >> 16) | (b & u32(0xFFFF0000))
        for c, v in ((0, lo), (1, hi)):
            for half in range(2):
                blk = c * (HB // 2) + half * 8
                view[pl.ds(blk * pitch + p, 8, stride=pitch), :] = v[half * 8:(half + 1) * 8, :]
        if zero is not None:
            t = lo | hi
            z = (t[0:8] | t[8:16]) & zero
            delay = DELAY_EVERY if delay is None else delay
            if delay and p % delay == delay - 1:
                z = pltpu.roll(z, 1, 1)
    return z


DELAY_EVERY = 3


def _mult(x, n):
    return x if isinstance(x, int) else pl.multiple_of(x, n)


def _b_deint_q(wq_raw, wq_d, j, zero=None, z=None, delay=None):
    return _b_deint(wq_raw, wq_d, PQ, _mult(j * 128, 128), _mult(j * 64, 64), zero, z, delay)


def _b_deint_kv(wukv_raw, wkv_d, j, zero=None, z=None, delay=None):
    return _b_deint(wukv_raw, wkv_d.at[j // 4], PK, _mult(j * 128, 128), _mult((j % 4) * 64, 64),
                    zero, z, delay)


def _b_qk(i, q_s, k_s):
    base = i * TQ
    q = _upk(q_s[base // 2:(base + TQ) // 2, :])
    s0 = _dot_nt(q, _upk(k_s[0:(base + 128) // 2, :]))
    sd = [_dot_nt(q[t * 128:], _upk(k_s[(base + t * 128) // 2:(base + (t + 1) * 128) // 2, :]))
          for t in range(1, RT)]
    return s0, sd


def _b_softmax_pv(i, s0, sd, v_s, ctx_h):
    base = i * TQ
    row = jax.lax.broadcasted_iota(jnp.int32, (128, 128), 0)
    col = jax.lax.broadcasted_iota(jnp.int32, (128, 128), 1)
    tri = col <= row
    ps, ls = [], []
    for r in range(RT):
        parts = [s0[r * 128:(r + 1) * 128]]
        parts += [sd[t - 1][(r - t) * 128:(r - t + 1) * 128] for t in range(1, r + 1)]
        sr = jnp.concatenate(parts, axis=1) if len(parts) > 1 else parts[0]
        lr = base + (r + 1) * 128
        dg = jnp.where(tri, sr[:, lr - 128:], NEG)
        sr = jnp.concatenate([sr[:, :lr - 128], dg], axis=1) if lr > 128 else dg
        m = jnp.max(sr, axis=1, keepdims=True)
        p = jnp.exp2(sr - m)
        xs = [p[:, j * 128:(j + 1) * 128] for j in range(lr // 128)]
        grp = []
        for k in range(0, len(xs), 4):
            acc = xs[k]
            for y in xs[k + 1:k + 4]:
                acc = acc + y
            grp.append(acc)
        part = _tree(grp, jnp.add)
        ls.append(jnp.sum(part, axis=1, keepdims=True))
        ps.append(p)
    p0 = jnp.concatenate([p[:, :base + 128] for p in ps], axis=0)
    o = jnp.dot(p0.astype(bf16), _upk(v_s[0:(base + 128) // 2, :]), preferred_element_type=f32)
    os_ = [o[r * 128:(r + 1) * 128] for r in range(RT)]
    for t in range(1, RT):
        lo, hi = base + t * 128, base + (t + 1) * 128
        pt = [ps[r][:, lo:hi] for r in range(t, RT)]
        pt = jnp.concatenate(pt, axis=0) if len(pt) > 1 else pt[0]
        ot = jnp.dot(pt.astype(bf16), _upk(v_s[lo // 2:hi // 2, :]), preferred_element_type=f32)
        for r in range(t, RT):
            os_[r] = os_[r] + ot[(r - t) * 128:(r - t + 1) * 128]
    for r in range(RT):
        lo = base + r * 128
        ctx_h[lo // 2:(lo + 128) // 2, :] = _pk((os_[r] * _recip(ls[r])).astype(bf16))


def _b_head(h, xb, ckv, wq_d, wkv_d, q_s, k_s, v_s, ctx):
    blk = _head_block(h)
    wq = _upk(wq_d[pl.ds(blk * PQ, DM // 2), :])
    q = jnp.dot(xb[...], wq, preferred_element_type=f32) * SCALE_B
    q_s[...] = _pk(q.astype(bf16))
    wkv = jnp.concatenate([_upk(wkv_d[t, pl.ds(blk * PK, DC // 2), :]) for t in range(2)], axis=1)
    kv = jnp.dot(ckv[...], wkv, preferred_element_type=f32)
    k_s[...] = _pk(kv[:, :DB].astype(bf16))
    v_s[...] = _pk(kv[:, DB:].astype(bf16))
    ctx_h = ctx.at[h]
    order = list(range(NQ))[::-1]
    nx = _b_qk(order[0], q_s, k_s)
    for n, i in enumerate(order):
        cu = nx
        if n + 1 < NQ:
            nx = _b_qk(order[n + 1], q_s, k_s)
        _b_softmax_pv(i, cu[0], cu[1], v_s, ctx_h)


XC = 256
NU = 8
WCH = (4, 2, 2)
SEM_W = (0, 4, 6)
SEM_WOA, SEM_CKV, SEM_XB, SEM_WOB, SEM_XA = 8, 9, 10, 11, 12
SEM_WQ = SEM_XA + S // XC
SEM_WUKV = SEM_WQ + NU
NSEM_IN = SEM_WUKV + NU


def _kernel(xa_hbm, wqkv_hbm, woa_hbm, xb_hbm, ckv_hbm, wq_hbm, wuk_hbm, wuv_hbm, wob_hbm,
            out_hbm,
            xa, wqkv, woa, wt, wop, q0, k0, v0, q1, k1, v1, ob0, ob1, stage,
            xb, ckv, wq, wukv, wob, wq_d, wkv_d, q_s, k_s, v_s, ctx,
            zero_s, sem_in, sem_a, sem_b):
    def in_copy(idx, src, dst):
        return pltpu.make_async_copy(src, dst, sem_in.at[idx])

    def rows(j, n):
        return pl.ds(j * n if isinstance(j, int) else pl.multiple_of(j * n, n), n)

    def c_w(t, c):
        r = rows(c, DM // WCH[t])
        cols = slice(t * DM, (t + 1) * DM)
        return in_copy(SEM_W[t] + c, wqkv_hbm.at[r, cols], wqkv.at[r, cols])

    def c_xa(j):
        return in_copy(SEM_XA + j, xa_hbm.at[rows(j, XC)], xa.at[rows(j, XC)])

    c_woa = in_copy(SEM_WOA, woa_hbm, woa)

    def c_wq(j):
        return in_copy(SEM_WQ + j, wq_hbm.at[rows(j, 128)], wq.at[rows(j, 128)])

    def c_wukv_start(j):
        src = wuk_hbm.at[rows(j, 128)] if j < 4 else wuv_hbm.at[rows(j - 4, 128)]
        in_copy(SEM_WUKV + j, src, wukv.at[rows(j, 128)]).start()

    def c_wukv_wait(j):
        dst = wukv.at[rows(j, 128)]
        in_copy(SEM_WUKV + j, dst, dst).wait()

    c_ckv = in_copy(SEM_CKV, ckv_hbm, ckv)
    c_xb = in_copy(SEM_XB, xb_hbm, xb)
    c_wob = in_copy(SEM_WOB, wob_hbm, wob)

    def a_out_copy(i):
        return pltpu.make_async_copy(stage.at[rows(i, TA), :],
                                     out_hbm.at[rows(i, TA), 0:DM], sem_a.at[i])

    def b_out_copy(i):
        return pltpu.make_async_copy(stage.at[rows(i, TO), :],
                                     out_hbm.at[rows(i, TO), DM:2 * DM], sem_b.at[i])

    for c in range(WCH[0]):
        c_w(0, c).start()
    c_xa(0).start()
    for t in (1, 2):
        for c in range(WCH[t]):
            c_w(t, c).start()
    c_woa.start()
    for j in range(NU):
        if j + 1 < S // XC:
            c_xa(j + 1).start()
        c_wq(j).start()
        c_wukv_start(j)
    for c in (c_ckv, c_xb, c_wob):
        c.start()
    zero_s[0] = jnp.uint32(0)

    bufs = [(q0, k0, v0), (q1, k1, v1)]
    obuf = [ob0, ob1]
    k0[:, 0:HALO, :] = jnp.zeros((8, HALO, 128), f32)
    v0[:, 0:HALO, :] = jnp.zeros((8, HALO, 128), f32)
    proj = functools.partial(_a_proj_third, xa, wt)
    for c in range(4):
        c_w(0, c).wait()
        _prep_wt(wqkv, 0, wt, range(2 * c, 2 * c + 2))
    c_xa(0).wait()
    proj(0, 0, bufs[0])

    def piece(blk, t, half):
        _a_proj_piece(xa, wt, blk * TA, t * (DM // PC) + half, bufs[blk])

    c_w(1, 0).wait()
    piece(1, 0, 0)
    _prep_wt(wqkv, 1, wt, range(0, 4))
    c_w(1, 1).wait()
    piece(1, 0, 1)
    _prep_wt(wqkv, 1, wt, range(4, 8))
    proj(0, 1, bufs[0])
    c_w(2, 0).wait()
    piece(1, 1, 0)
    _prep_wt(wqkv, 2, wt, range(0, 4))
    c_w(2, 1).wait()
    piece(1, 1, 1)
    _prep_wt(wqkv, 2, wt, range(4, 8))
    proj(0, 2, bufs[0])
    c_woa.wait()
    for t in (1, 2):
        _a_halo(bufs[0], bufs[1], t)
    _a_attn(bufs, obuf, 0, 0)
    proj(1, 2, bufs[1])
    _prep_wo(woa, wop)

    st = functools.partial(_a_stage, xa, wt, wop, stage, a_out_copy, bufs, obuf)

    def a_body(j, carry):
        c_xa(j + 1).wait()
        c_wq(j).wait()
        c_wukv_wait(j)
        zero = jnp.full((8, 128), zero_s[0], u32)
        z = _b_deint_q(wq, wq_d, j, zero)
        _b_deint_kv(wukv, wkv_d, j, zero, z)
        st(2 * j + 1, 1, True)
        st(2 * j + 2, 0, True)
        return carry

    jax.lax.fori_loop(0, (NA - 2) // 2, a_body, 0)

    c_wq(NU - 1).wait()
    c_wukv_wait(NU - 1)
    zero = jnp.full((8, 128), zero_s[0], u32)

    def last_units():
        z = _b_deint_q(wq, wq_d, NU - 1, zero, None, 0)
        _b_deint_kv(wukv, wkv_d, NU - 1, zero, z, 0)

    st(NA - 1, 1, False, side=[last_units])
    _a_out(wop, stage, a_out_copy, obuf, NA - 1, 1)
    c_ckv.wait()
    c_xb.wait()

    def b_body(h, carry):
        _b_head(h, xb, ckv, wq_d, wkv_d, q_s, k_s, v_s, ctx)
        return carry

    jax.lax.fori_loop(0, HB, b_body, 0)

    c_wob.wait()
    for i in range(NA):
        a_out_copy(i).wait()

    def o_body(i, carry):
        r2 = pl.multiple_of(i * (TO // 2), TO // 2)
        lhs = jnp.concatenate(
            [_upk(ctx[h, pl.ds(r2, TO // 2), :]) for h in range(HB)], axis=1)
        y = jnp.dot(lhs, wob[...], preferred_element_type=f32)
        stage[pl.ds(pl.multiple_of(i * TO, TO), TO), :] = y.astype(bf16)
        b_out_copy(i).start()
        return carry

    jax.lax.fori_loop(0, S // TO, o_body, 0)
    for i in range(S // TO):
        b_out_copy(i).wait()


@jax.jit
def pallas_concat_heads__sliding_local_dilated__compressed_kv_cla__prompt_kernel(
    A_x: jax.Array,
    A_wqkv: jax.Array,
    A_wo: jax.Array,
    B_x: jax.Array,
    B_c_kv: jax.Array,
    B_w_q: jax.Array,
    B_w_uk: jax.Array,
    B_w_uv: jax.Array,
    B_w_o: jax.Array,
):
    V = pltpu.VMEM
    slab = lambda n: V((8, n, 128), f32)
    scratch = [
        V((S, DM), bf16),
        V((DM, 3 * DM), bf16),
        V((DM, DM), bf16),
        V((DM // 128, 3 * NW, 128), u32),
        V((DM // 128, NW, 128), u32),
        slab(TA), slab(TA + HALO), slab(TA + HALO),
        slab(TA), slab(TA + HALO), slab(TA + HALO),
        V((TA // 2, DM), u32), V((TA // 2, DM), u32),
        V((S, DM), bf16),
        V((S, DM), bf16),
        V((S, DC), bf16),
        V((DM, HB, DB), bf16),
        V((2 * DC, HB, DB), bf16),
        V((HB * DB, DM), bf16),
        V((HB * PQ, DB), u32),
        V((2, HB * PK, DB), u32),
        V((S // 2, DB), u32), V((S // 2, DB), u32), V((S // 2, DB), u32),
        V((HB, S // 2, DB), u32),
        pltpu.SMEM((1,), u32),
        pltpu.SemaphoreType.DMA((NSEM_IN,)),
        pltpu.SemaphoreType.DMA((NA,)),
        pltpu.SemaphoreType.DMA((S // TO,)),
    ]
    any_spec = pl.BlockSpec(memory_space=pl.ANY)
    out = pl.pallas_call(
        _kernel,
        out_shape=jax.ShapeDtypeStruct((S, 2 * DM), bf16),
        in_specs=[any_spec] * 9,
        out_specs=any_spec,
        scratch_shapes=scratch,
        compiler_params=pltpu.CompilerParams(vmem_limit_bytes=120 * 1024 * 1024),
    )(
        A_x.reshape(S, DM), A_wqkv, A_wo,
        B_x.reshape(S, DM), B_c_kv.reshape(S, DC), B_w_q, B_w_uk, B_w_uv,
        B_w_o.reshape(HB * DB, DM),
    )
    return out.reshape(1, S, 2 * DM)
```

```python
import functools
import math

import jax
import jax.numpy as jnp
import jax.experimental.pallas as pl
import jax.experimental.pallas.tpu as pltpu

bf16 = jnp.bfloat16
f32 = jnp.float32
u32 = jnp.uint32

NEG = -1e9
LOG2E = math.log2(math.e)
NT = (((1,), (1,)), ((), ()))

S = 2048
DM = 1024
HA, DH, WIN, DIL = 32, 32, 8, 2
TA = 128
NA = S // TA
HALO = 16
RC = 64
PC = 512
SCALE_A = DH ** -0.5 * LOG2E
HB, DB, DC = 32, 128, 512
TQ = 256
NQ = S // TQ
RT = TQ // 128
SCALE_B = DB ** -0.5 * LOG2E
TO = 256


def _pk(x):
    return pltpu.bitcast(x, u32)


def _upk(x):
    return pltpu.bitcast(x, bf16)


def _tree(xs, op):
    xs = list(xs)
    while len(xs) > 1:
        xs = [op(xs[k], xs[k + 1]) if k + 1 < len(xs) else xs[k] for k in range(0, len(xs), 2)]
    return xs[0]


def _dot_nt(a, b):
    return jax.lax.dot_general(a, b, NT, preferred_element_type=f32)


def _recip(l):
    return pl.reciprocal(l, approx=False, full_range=False)


PW = HA // 2 + 1
NW = DH * PW


def _repack_heads(u, dst, base):
    for hp in range(HA // 2):
        a = u[(2 * hp) * 16:(2 * hp + 1) * 16]
        b = u[(2 * hp + 1) * 16:(2 * hp + 2) * 16]
        lo = (a & u32(0xFFFF)) | (b << 16)
        hi = (a >> 16) | (b & u32(0xFFFF0000))
        for k, v in enumerate((lo[0:8], lo[8:16], hi[0:8], hi[8:16])):
            dst[pl.ds(base + k * 8 * PW + hp, 8, stride=PW), :] = v


def _load_slots(src, base, s0, s1):
    return jnp.concatenate([src[base + d * PW:base + d * PW + 16, :] for d in range(s0, s1)], axis=0)


def _prep_wt(w_ref, t, wt_ref, mcs=range(DM // 128)):
    for mc in mcs:
        blk = w_ref[mc * 128:(mc + 1) * 128, t * DM:(t + 1) * DM]
        _repack_heads(_pk(blk.T), wt_ref.at[mc], t * NW)


def _prep_wo(wo_ref, wop_ref):
    for nc in range(DM // 128):
        _repack_heads(_pk(wo_ref[:, nc * 128:(nc + 1) * 128]), wop_ref.at[nc], 0)


def _a_proj_piece(x_ref, wt_ref, r0, n, nxt):
    x = x_ref[pl.ds(r0, TA), :]
    t, s0 = (n * PC) // DM, ((n * PC) % DM) // HA
    w = jnp.concatenate([_load_slots(wt_ref.at[mc], t * NW, s0, s0 + PC // HA)
                         for mc in range(DM // 128)], axis=1)
    y = _dot_nt(x, _upk(w))
    for j in range(PC // 128):
        col = n * PC + j * 128
        t, g = col // DM, (col % DM) // 128
        blk = y[:, j * 128:(j + 1) * 128]
        if t == 0:
            nxt[0][g, :, :] = blk * SCALE_A
        else:
            nxt[t][g, HALO:HALO + TA, :] = blk


def _a_attn_chunk(bufs, r0, c, o_ref):
    qv, kv, vv = bufs
    a = c * RC
    pos = r0 + a + jax.lax.broadcasted_iota(jnp.int32, (RC, 128), 0)
    q = [qv[g, a:a + RC, :] for g in range(8)]
    s = []
    for w in range(WIN):
        o = HALO + a - DIL * w
        acc = q[0] * kv[0, o:o + RC, :]
        for g in range(1, 8):
            acc = acc + q[g] * kv[g, o:o + RC, :]
        acc = acc + pltpu.roll(acc, 64, 1)
        acc = acc + pltpu.roll(acc, 32, 1)
        if w > 0:
            acc = jnp.where(pos >= DIL * w, acc, NEG)
        s.append(acc)
    m = s[0]
    for w in range(1, WIN):
        m = jnp.maximum(m, s[w])
    e = [jnp.exp2(s[w] - m) for w in range(WIN)]
    l = e[0]
    for w in range(1, WIN):
        l = l + e[w]
    inv = _recip(l)
    cols = []
    for g in range(8):
        acc = e[0] * vv[g, HALO + a:HALO + a + RC, :]
        for w in range(1, WIN):
            o = HALO + a - DIL * w
            acc = acc + e[w] * vv[g, o:o + RC, :]
        cols.append(acc * inv)
    o_ref[a // 2:(a + RC) // 2, :] = _pk(jnp.concatenate(cols, axis=1).astype(bf16))


def _a_out_piece(o_ref, wop_ref, stage_ref, r0, n):
    w = jnp.concatenate([_load_slots(wop_ref.at[nc], 0, 0, DH)
                         for nc in range(n * PC // 128, (n + 1) * PC // 128)], axis=1)
    y = jnp.dot(_upk(o_ref[...]), _upk(w), preferred_element_type=f32)
    stage_ref[pl.ds(r0, TA), n * PC:(n + 1) * PC] = y.astype(bf16)


def _a_halo(cur, nxt, t):
    nxt[t][:, 0:HALO, :] = cur[t][:, TA:TA + HALO, :]


def _a_proj_third(x_ref, wt_ref, blk, t, dst):
    rn = blk * TA
    if not isinstance(rn, int):
        rn = pl.multiple_of(rn, TA)
    for n in range(t * DM // PC, (t + 1) * DM // PC):
        _a_proj_piece(x_ref, wt_ref, rn, n, dst)


def _a_attn(bufs, obuf, i, par):
    for c in range(TA // RC):
        _a_attn_chunk(bufs[par], i * TA, c, obuf[par])


def _a_out(wop_ref, stage_ref, out_copy, obuf, i, par):
    rp = i * TA
    if not isinstance(rp, int):
        rp = pl.multiple_of(rp, TA)
    for n in range(DM // PC):
        _a_out_piece(obuf[par], wop_ref, stage_ref, rp, n)
    out_copy(i).start()


def _a_stage(x_ref, wt_ref, wop_ref, stage_ref, out_copy, bufs, obuf,
             i, par, do_proj, side=()):
    if do_proj:
        for t in (1, 2):
            _a_halo(bufs[par], bufs[1 - par], t)
    _a_attn(bufs, obuf, i, par)
    mm = []
    if do_proj:
        rn = (i + 1) * TA
        if not isinstance(rn, int):
            rn = pl.multiple_of(rn, TA)
        mm += [functools.partial(_a_proj_piece, x_ref, wt_ref, rn, n, bufs[1 - par])
               for n in range(3 * DM // PC)]
    rp = (i - 1) * TA
    if not isinstance(rp, int):
        rp = pl.multiple_of(rp, TA)
    mm += [functools.partial(_a_out_piece, obuf[1 - par], wop_ref, stage_ref, rp, n)
           for n in range(DM // PC)]
    for f in side:
        f()
    for f in mm:
        f()
    out_copy(i - 1).start()


PK = DC // 2 + 1
NU = 16


def _b_deint(raw, dst, pitch, r0, p0, zero=None, z=None, delay=None):
    span = (HB - 1) * pitch + 64
    view = dst.at[pl.ds(p0, span), :]
    src = raw.at[pl.ds(r0, 128)]
    for p in range(64):
        x = pltpu.bitcast(src[2 * p:2 * p + 2], u32)
        a, b = x[0], x[1]
        if z is not None:
            a = a | jnp.concatenate([z, z], axis=0)
        lo = (a & u32(0xFFFF)) | (b << 16)
        hi = (a >> 16) | (b & u32(0xFFFF0000))
        for c, v in ((0, lo), (1, hi)):
            for half in range(2):
                blk = c * (HB // 2) + half * 8
                view[pl.ds(blk * pitch + p, 8, stride=pitch), :] = v[half * 8:(half + 1) * 8, :]
        if zero is not None:
            t = lo | hi
            z = (t[0:8] | t[8:16]) & zero
            delay = DELAY_EVERY if delay is None else delay
            if delay and p % delay == delay - 1:
                z = pltpu.roll(z, 1, 1)
    return z


DELAY_EVERY = 3


def _mult(x, n):
    return x if isinstance(x, int) else pl.multiple_of(x, n)


def _b_deint_unit(wraw, wd, u, zero=None, z=None, delay=None):
    return _b_deint(wraw, wd.at[u // 4], PK, _mult(u * 128, 128), _mult((u % 4) * 64, 64),
                    zero, z, delay)


def _b_qk(i, q_s, k_s):
    base = i * TQ
    q = _upk(q_s[base // 2:(base + TQ) // 2, :])
    s0 = _dot_nt(q, _upk(k_s[0:(base + 128) // 2, :]))
    sd = [_dot_nt(q[t * 128:], _upk(k_s[(base + t * 128) // 2:(base + (t + 1) * 128) // 2, :]))
          for t in range(1, RT)]
    return s0, sd


def _b_softmax_pv(i, s0, sd, v_s, ctx_h):
    base = i * TQ
    row = jax.lax.broadcasted_iota(jnp.int32, (128, 128), 0)
    col = jax.lax.broadcasted_iota(jnp.int32, (128, 128), 1)
    tri = col <= row
    ps, ls = [], []
    for r in range(RT):
        parts = [s0[r * 128:(r + 1) * 128]]
        parts += [sd[t - 1][(r - t) * 128:(r - t + 1) * 128] for t in range(1, r + 1)]
        sr = jnp.concatenate(parts, axis=1) if len(parts) > 1 else parts[0]
        lr = base + (r + 1) * 128
        dg = jnp.where(tri, sr[:, lr - 128:], NEG)
        sr = jnp.concatenate([sr[:, :lr - 128], dg], axis=1) if lr > 128 else dg
        m = jnp.max(sr, axis=1, keepdims=True)
        p = jnp.exp2(sr - m)
        xs = [p[:, j * 128:(j + 1) * 128] for j in range(lr // 128)]
        grp = []
        for k in range(0, len(xs), 4):
            acc = xs[k]
            for y in xs[k + 1:k + 4]:
                acc = acc + y
            grp.append(acc)
        part = _tree(grp, jnp.add)
        ls.append(jnp.sum(part, axis=1, keepdims=True))
        ps.append(p)
    p0 = jnp.concatenate([p[:, :base + 128] for p in ps], axis=0)
    o = jnp.dot(p0.astype(bf16), _upk(v_s[0:(base + 128) // 2, :]), preferred_element_type=f32)
    os_ = [o[r * 128:(r + 1) * 128] for r in range(RT)]
    for t in range(1, RT):
        lo, hi = base + t * 128, base + (t + 1) * 128
        pt = [ps[r][:, lo:hi] for r in range(t, RT)]
        pt = jnp.concatenate(pt, axis=0) if len(pt) > 1 else pt[0]
        ot = jnp.dot(pt.astype(bf16), _upk(v_s[lo // 2:hi // 2, :]), preferred_element_type=f32)
        for r in range(t, RT):
            os_[r] = os_[r] + ot[(r - t) * 128:(r - t + 1) * 128]
    for r in range(RT):
        lo = base + r * 128
        ctx_h[lo // 2:(lo + 128) // 2, :] = _pk((os_[r] * _recip(ls[r])).astype(bf16))


def _b_head(b, xb, ckv, wd, q_s, k_s, v_s, ctx):
    h = (b % (HB // 2)) * 2 + b // (HB // 2)
    blk = pl.ds(b * PK, DC // 2)
    wq = _upk(jnp.concatenate([wd[0, blk, :], wd[1, blk, :]], axis=0))
    q = jnp.dot(xb[...], wq, preferred_element_type=f32) * SCALE_B
    q_s[...] = _pk(q.astype(bf16))
    wkv = _upk(jnp.concatenate([wd[2, blk, :], wd[3, blk, :]], axis=1))
    kv = jnp.dot(ckv[...], wkv, preferred_element_type=f32)
    k_s[...] = _pk(kv[:, :DB].astype(bf16))
    v_s[...] = _pk(kv[:, DB:].astype(bf16))
    ctx_h = ctx.at[h]
    order = list(range(NQ))[::-1]
    nx = _b_qk(order[0], q_s, k_s)
    for n, i in enumerate(order):
        cu = nx
        if n + 1 < NQ:
            nx = _b_qk(order[n + 1], q_s, k_s)
        _b_softmax_pv(i, cu[0], cu[1], v_s, ctx_h)


XC = 256
WCH = (4, 2, 2)
SEM_W = (0, 4, 6)
SEM_WOA, SEM_CKV, SEM_XB, SEM_WOB, SEM_XA = 8, 9, 10, 11, 12
SEM_WU = SEM_XA + S // XC
NSEM_IN = SEM_WU + NU


def _kernel(xa_hbm, wqkv_hbm, woa_hbm, xb_hbm, ckv_hbm, wq_hbm, wuk_hbm, wuv_hbm, wob_hbm,
            out_hbm,
            xa, wqkv, woa, wt, wop, q0, k0, v0, q1, k1, v1, ob0, ob1, stage,
            xb, ckv, wraw, wob, wd, q_s, k_s, v_s, ctx,
            zero_s, sem_in, sem_a, sem_b):
    def in_copy(idx, src, dst):
        return pltpu.make_async_copy(src, dst, sem_in.at[idx])

    def rows(j, n):
        return pl.ds(j * n if isinstance(j, int) else pl.multiple_of(j * n, n), n)

    def c_w(t, c):
        r = rows(c, DM // WCH[t])
        cols = slice(t * DM, (t + 1) * DM)
        return in_copy(SEM_W[t] + c, wqkv_hbm.at[r, cols], wqkv.at[r, cols])

    def c_xa(j):
        return in_copy(SEM_XA + j, xa_hbm.at[rows(j, XC)], xa.at[rows(j, XC)])

    c_woa = in_copy(SEM_WOA, woa_hbm, woa)

    def c_wu_start(u):
        if u < 8:
            src = wq_hbm.at[rows(u, 128)]
        elif u < 12:
            src = wuk_hbm.at[rows(u - 8, 128)]
        else:
            src = wuv_hbm.at[rows(u - 12, 128)]
        in_copy(SEM_WU + u, src, wraw.at[rows(u, 128)]).start()

    def c_wu_wait(u):
        dst = wraw.at[rows(u, 128)]
        in_copy(SEM_WU + u, dst, dst).wait()

    c_ckv = in_copy(SEM_CKV, ckv_hbm, ckv)
    c_xb = in_copy(SEM_XB, xb_hbm, xb)
    c_wob = in_copy(SEM_WOB, wob_hbm, wob)

    def a_out_copy(i):
        return pltpu.make_async_copy(stage.at[rows(i, TA), :],
                                     out_hbm.at[rows(i, TA), 0:DM], sem_a.at[i])

    def b_out_copy(i):
        return pltpu.make_async_copy(stage.at[rows(i, TO), :],
                                     out_hbm.at[rows(i, TO), DM:2 * DM], sem_b.at[i])

    for c in range(WCH[0]):
        c_w(0, c).start()
    c_xa(0).start()
    for t in (1, 2):
        for c in range(WCH[t]):
            c_w(t, c).start()
    c_woa.start()
    for j in range(S // XC - 1):
        c_xa(j + 1).start()
        if j > 0:
            c_wu_start(2 * j - 1)
        c_wu_start(2 * j)
    for u in range(2 * (S // XC - 2) + 1, NU):
        c_wu_start(u)
    for c in (c_ckv, c_xb, c_wob):
        c.start()
    zero_s[0] = jnp.uint32(0)

    bufs = [(q0, k0, v0), (q1, k1, v1)]
    obuf = [ob0, ob1]
    k0[:, 0:HALO, :] = jnp.zeros((8, HALO, 128), f32)
    v0[:, 0:HALO, :] = jnp.zeros((8, HALO, 128), f32)
    proj = functools.partial(_a_proj_third, xa, wt)
    for c in range(4):
        c_w(0, c).wait()
        _prep_wt(wqkv, 0, wt, range(2 * c, 2 * c + 2))
    c_xa(0).wait()
    proj(0, 0, bufs[0])

    def piece(blk, t, half):
        _a_proj_piece(xa, wt, blk * TA, t * (DM // PC) + half, bufs[blk])

    c_w(1, 0).wait()
    piece(1, 0, 0)
    _prep_wt(wqkv, 1, wt, range(0, 4))
    c_w(1, 1).wait()
    piece(1, 0, 1)
    _prep_wt(wqkv, 1, wt, range(4, 8))
    proj(0, 1, bufs[0])
    c_w(2, 0).wait()
    piece(1, 1, 0)
    _prep_wt(wqkv, 2, wt, range(0, 4))
    c_w(2, 1).wait()
    piece(1, 1, 1)
    _prep_wt(wqkv, 2, wt, range(4, 8))
    proj(0, 2, bufs[0])
    c_woa.wait()
    for t in (1, 2):
        _a_halo(bufs[0], bufs[1], t)
    _a_attn(bufs, obuf, 0, 0)
    proj(1, 2, bufs[1])
    _prep_wo(woa, wop)

    st = functools.partial(_a_stage, xa, wt, wop, stage, a_out_copy, bufs, obuf)

    def a_body(j, carry):
        c_xa(j + 1).wait()

        @pl.when(j > 0)
        def _():
            c_wu_wait(2 * j - 1)

        c_wu_wait(2 * j)
        zero = jnp.full((8, 128), zero_s[0], u32)
        z = _b_deint_unit(wraw, wd, jnp.maximum(2 * j - 1, 0), zero)
        _b_deint_unit(wraw, wd, 2 * j, zero, z)
        st(2 * j + 1, 1, True)
        st(2 * j + 2, 0, True)
        return carry

    jax.lax.fori_loop(0, (NA - 2) // 2, a_body, 0)

    for u in range(NU - 3, NU):
        c_wu_wait(u)
    zero = jnp.full((8, 128), zero_s[0], u32)

    def last_units():
        z = _b_deint_unit(wraw, wd, NU - 3, zero, None, 0)
        _b_deint_unit(wraw, wd, NU - 2, zero, z, 0)
        _b_deint_unit(wraw, wd, NU - 1, zero, None, 0)

    st(NA - 1, 1, False, side=[last_units])
    _a_out(wop, stage, a_out_copy, obuf, NA - 1, 1)
    c_ckv.wait()
    c_xb.wait()

    def b_body(h, carry):
        _b_head(h, xb, ckv, wd, q_s, k_s, v_s, ctx)
        return carry

    jax.lax.fori_loop(0, HB, b_body, 0)

    c_wob.wait()
    for i in range(NA):
        a_out_copy(i).wait()

    def o_body(i, carry):
        r2 = pl.multiple_of(i * (TO // 2), TO // 2)
        lhs = jnp.concatenate(
            [_upk(ctx[h, pl.ds(r2, TO // 2), :]) for h in range(HB)], axis=1)
        y = jnp.dot(lhs, wob[...], preferred_element_type=f32)
        stage[pl.ds(pl.multiple_of(i * TO, TO), TO), :] = y.astype(bf16)
        b_out_copy(i).start()
        return carry

    jax.lax.fori_loop(0, S // TO, o_body, 0)
    for i in range(S // TO):
        b_out_copy(i).wait()


@jax.jit
def pallas_concat_heads__sliding_local_dilated__compressed_kv_cla__prompt_kernel(
    A_x: jax.Array,
    A_wqkv: jax.Array,
    A_wo: jax.Array,
    B_x: jax.Array,
    B_c_kv: jax.Array,
    B_w_q: jax.Array,
    B_w_uk: jax.Array,
    B_w_uv: jax.Array,
    B_w_o: jax.Array,
):
    V = pltpu.VMEM
    slab = lambda n: V((8, n, 128), f32)
    scratch = [
        V((S, DM), bf16),
        V((DM, 3 * DM), bf16),
        V((DM, DM), bf16),
        V((DM // 128, 3 * NW, 128), u32),
        V((DM // 128, NW, 128), u32),
        slab(TA), slab(TA + HALO), slab(TA + HALO),
        slab(TA), slab(TA + HALO), slab(TA + HALO),
        V((TA // 2, DM), u32), V((TA // 2, DM), u32),
        V((S, DM), bf16),
        V((S, DM), bf16),
        V((S, DC), bf16),
        V((DM + 2 * DC, HB, DB), bf16),
        V((HB * DB, DM), bf16),
        V((4, HB * PK, DB), u32),
        V((S // 2, DB), u32), V((S // 2, DB), u32), V((S // 2, DB), u32),
        V((HB, S // 2, DB), u32),
        pltpu.SMEM((1,), u32),
        pltpu.SemaphoreType.DMA((NSEM_IN,)),
        pltpu.SemaphoreType.DMA((NA,)),
        pltpu.SemaphoreType.DMA((S // TO,)),
    ]
    any_spec = pl.BlockSpec(memory_space=pl.ANY)
    out = pl.pallas_call(
        _kernel,
        out_shape=jax.ShapeDtypeStruct((S, 2 * DM), bf16),
        in_specs=[any_spec] * 9,
        out_specs=any_spec,
        scratch_shapes=scratch,
        compiler_params=pltpu.CompilerParams(vmem_limit_bytes=120 * 1024 * 1024,
                                             disable_bounds_checks=True),
    )(
        A_x.reshape(S, DM), A_wqkv, A_wo,
        B_x.reshape(S, DM), B_c_kv.reshape(S, DC), B_w_q, B_w_uk, B_w_uv,
        B_w_o.reshape(HB * DB, DM),
    )
    return out.reshape(1, S, 2 * DM)
```

```python
import functools
import math

import jax
import jax.numpy as jnp
import jax.experimental.pallas as pl
import jax.experimental.pallas.tpu as pltpu

bf16 = jnp.bfloat16
f32 = jnp.float32
u32 = jnp.uint32

NEG = -1e9
LOG2E = math.log2(math.e)
NT = (((1,), (1,)), ((), ()))

S = 2048
DM = 1024
HA, DH, WIN, DIL = 32, 32, 8, 2
TA = 128
NA = S // TA
HALO = 16
RC = 64
PC = 512
SCALE_A = DH ** -0.5 * LOG2E
HB, DB, DC = 32, 128, 512
TQ = 256
NQ = S // TQ
RT = TQ // 128
SCALE_B = DB ** -0.5 * LOG2E
TO = 256


def _pk(x):
    return pltpu.bitcast(x, u32)


def _upk(x):
    return pltpu.bitcast(x, bf16)


def _tree(xs, op):
    xs = list(xs)
    while len(xs) > 1:
        xs = [op(xs[k], xs[k + 1]) if k + 1 < len(xs) else xs[k] for k in range(0, len(xs), 2)]
    return xs[0]


def _dot_nt(a, b):
    return jax.lax.dot_general(a, b, NT, preferred_element_type=f32)


def _recip(l):
    return pl.reciprocal(l, approx=False, full_range=False)


PW = HA // 2 + 1
NW = DH * PW


def _repack_heads(u, dst, base):
    for hp in range(HA // 2):
        a = u[(2 * hp) * 16:(2 * hp + 1) * 16]
        b = u[(2 * hp + 1) * 16:(2 * hp + 2) * 16]
        lo = (a & u32(0xFFFF)) | (b << 16)
        hi = (a >> 16) | (b & u32(0xFFFF0000))
        for k, v in enumerate((lo[0:8], lo[8:16], hi[0:8], hi[8:16])):
            dst[pl.ds(base + k * 8 * PW + hp, 8, stride=PW), :] = v


def _load_slots(src, base, s0, s1):
    return jnp.concatenate([src[base + d * PW:base + d * PW + 16, :] for d in range(s0, s1)], axis=0)


def _prep_wt(w_ref, t, wt_ref, mcs=range(DM // 128)):
    for mc in mcs:
        blk = w_ref[mc * 128:(mc + 1) * 128, t * DM:(t + 1) * DM]
        _repack_heads(_pk(blk.T), wt_ref.at[mc], t * NW)


def _prep_wo(wo_ref, wop_ref):
    for nc in range(DM // 128):
        _repack_heads(_pk(wo_ref[:, nc * 128:(nc + 1) * 128]), wop_ref.at[nc], 0)


def _a_proj_piece(x_ref, wt_ref, r0, n, nxt):
    x = x_ref[pl.ds(r0, TA), :]
    t, s0 = (n * PC) // DM, ((n * PC) % DM) // HA
    w = jnp.concatenate([_load_slots(wt_ref.at[mc], t * NW, s0, s0 + PC // HA)
                         for mc in range(DM // 128)], axis=1)
    y = _dot_nt(x, _upk(w))
    for j in range(PC // 128):
        col = n * PC + j * 128
        t, g = col // DM, (col % DM) // 128
        blk = y[:, j * 128:(j + 1) * 128]
        if t == 0:
            nxt[0][g, :, :] = blk * SCALE_A
        else:
            nxt[t][g, HALO:HALO + TA, :] = blk


def _a_attn_chunk(bufs, r0, c, o_ref):
    qv, kv, vv = bufs
    a = c * RC
    pos = r0 + a + jax.lax.broadcasted_iota(jnp.int32, (RC, 128), 0)
    q = [qv[g, a:a + RC, :] for g in range(8)]
    s = []
    for w in range(WIN):
        o = HALO + a - DIL * w
        acc = q[0] * kv[0, o:o + RC, :]
        for g in range(1, 8):
            acc = acc + q[g] * kv[g, o:o + RC, :]
        acc = acc + pltpu.roll(acc, 64, 1)
        acc = acc + pltpu.roll(acc, 32, 1)
        if w > 0:
            acc = jnp.where(pos >= DIL * w, acc, NEG)
        s.append(acc)
    m = s[0]
    for w in range(1, WIN):
        m = jnp.maximum(m, s[w])
    e = [jnp.exp2(s[w] - m) for w in range(WIN)]
    l = e[0]
    for w in range(1, WIN):
        l = l + e[w]
    inv = _recip(l)
    cols = []
    for g in range(8):
        acc = e[0] * vv[g, HALO + a:HALO + a + RC, :]
        for w in range(1, WIN):
            o = HALO + a - DIL * w
            acc = acc + e[w] * vv[g, o:o + RC, :]
        cols.append(acc * inv)
    o_ref[a // 2:(a + RC) // 2, :] = _pk(jnp.concatenate(cols, axis=1).astype(bf16))


def _a_out_piece(o_ref, wop_ref, stage_ref, r0, n):
    w = jnp.concatenate([_load_slots(wop_ref.at[nc], 0, 0, DH)
                         for nc in range(n * PC // 128, (n + 1) * PC // 128)], axis=1)
    y = jnp.dot(_upk(o_ref[...]), _upk(w), preferred_element_type=f32)
    stage_ref[pl.ds(r0, TA), n * PC:(n + 1) * PC] = y.astype(bf16)


def _a_halo(cur, nxt, t):
    nxt[t][:, 0:HALO, :] = cur[t][:, TA:TA + HALO, :]


def _a_proj_third(x_ref, wt_ref, blk, t, dst):
    rn = blk * TA
    if not isinstance(rn, int):
        rn = pl.multiple_of(rn, TA)
    for n in range(t * DM // PC, (t + 1) * DM // PC):
        _a_proj_piece(x_ref, wt_ref, rn, n, dst)


def _a_attn(bufs, obuf, i, par):
    for c in range(TA // RC):
        _a_attn_chunk(bufs[par], i * TA, c, obuf[par])


def _a_out(wop_ref, stage_ref, out_copy, obuf, i, par):
    rp = i * TA
    if not isinstance(rp, int):
        rp = pl.multiple_of(rp, TA)
    for n in range(DM // PC):
        _a_out_piece(obuf[par], wop_ref, stage_ref, rp, n)
    out_copy(i).start()


def _a_stage(x_ref, wt_ref, wop_ref, stage_ref, out_copy, bufs, obuf,
             i, par, do_proj, side=()):
    if do_proj:
        for t in (1, 2):
            _a_halo(bufs[par], bufs[1 - par], t)
    _a_attn(bufs, obuf, i, par)
    mm = []
    if do_proj:
        rn = (i + 1) * TA
        if not isinstance(rn, int):
            rn = pl.multiple_of(rn, TA)
        mm += [functools.partial(_a_proj_piece, x_ref, wt_ref, rn, n, bufs[1 - par])
               for n in range(3 * DM // PC)]
    rp = (i - 1) * TA
    if not isinstance(rp, int):
        rp = pl.multiple_of(rp, TA)
    mm += [functools.partial(_a_out_piece, obuf[1 - par], wop_ref, stage_ref, rp, n)
           for n in range(DM // PC)]
    for f in side:
        f()
    for f in mm:
        f()
    out_copy(i - 1).start()


PK = DC // 2 + 1
NU = 16


def _b_deint(raw, dst, pitch, r0, p0, zero=None, z=None, delay=None):
    span = (HB - 1) * pitch + 64
    view = dst.at[pl.ds(p0, span), :]
    src = raw.at[pl.ds(r0, 128)]
    for p in range(64):
        x = pltpu.bitcast(src[2 * p:2 * p + 2], u32)
        a, b = x[0], x[1]
        if z is not None:
            a = a | jnp.concatenate([z, z], axis=0)
        lo = (a & u32(0xFFFF)) | (b << 16)
        hi = (a >> 16) | (b & u32(0xFFFF0000))
        for c, v in ((0, lo), (1, hi)):
            for half in range(2):
                blk = c * (HB // 2) + half * 8
                view[pl.ds(blk * pitch + p, 8, stride=pitch), :] = v[half * 8:(half + 1) * 8, :]
        if zero is not None:
            t = lo | hi
            z = (t[0:8] | t[8:16]) & zero
            delay = DELAY_EVERY if delay is None else delay
            if delay and p % delay == delay - 1:
                z = pltpu.roll(z, 1, 1)
    return z


DELAY_EVERY = 3


def _mult(x, n):
    return x if isinstance(x, int) else pl.multiple_of(x, n)


def _b_deint_unit(wraw, wd, u, zero=None, z=None, delay=None):
    return _b_deint(wraw, wd.at[u // 4], PK, _mult(u * 128, 128), _mult((u % 4) * 64, 64),
                    zero, z, delay)


def _b_qk(i, q_s, k_s):
    base = i * TQ
    q = _upk(q_s[base // 2:(base + TQ) // 2, :])
    s0 = _dot_nt(q, _upk(k_s[0:(base + 128) // 2, :]))
    sd = [_dot_nt(q[t * 128:], _upk(k_s[(base + t * 128) // 2:(base + (t + 1) * 128) // 2, :]))
          for t in range(1, RT)]
    return s0, sd


def _b_softmax_pv(i, s0, sd, v_s, ctx_h):
    base = i * TQ
    row = jax.lax.broadcasted_iota(jnp.int32, (128, 128), 0)
    col = jax.lax.broadcasted_iota(jnp.int32, (128, 128), 1)
    tri = col <= row
    ps, ls = [], []
    for r in range(RT):
        parts = [s0[r * 128:(r + 1) * 128]]
        parts += [sd[t - 1][(r - t) * 128:(r - t + 1) * 128] for t in range(1, r + 1)]
        sr = jnp.concatenate(parts, axis=1) if len(parts) > 1 else parts[0]
        lr = base + (r + 1) * 128
        dg = jnp.where(tri, sr[:, lr - 128:], NEG)
        sr = jnp.concatenate([sr[:, :lr - 128], dg], axis=1) if lr > 128 else dg
        m = jnp.max(sr, axis=1, keepdims=True)
        p = jnp.exp2(sr - m)
        xs = [p[:, j * 128:(j + 1) * 128] for j in range(lr // 128)]
        grp = []
        for k in range(0, len(xs), 4):
            acc = xs[k]
            for y in xs[k + 1:k + 4]:
                acc = acc + y
            grp.append(acc)
        part = _tree(grp, jnp.add)
        ls.append(jnp.sum(part, axis=1, keepdims=True))
        ps.append(p)
    p0 = jnp.concatenate([p[:, :base + 128] for p in ps], axis=0)
    o = jnp.dot(p0.astype(bf16), _upk(v_s[0:(base + 128) // 2, :]), preferred_element_type=f32)
    os_ = [o[r * 128:(r + 1) * 128] for r in range(RT)]
    for t in range(1, RT):
        lo, hi = base + t * 128, base + (t + 1) * 128
        pt = [ps[r][:, lo:hi] for r in range(t, RT)]
        pt = jnp.concatenate(pt, axis=0) if len(pt) > 1 else pt[0]
        ot = jnp.dot(pt.astype(bf16), _upk(v_s[lo // 2:hi // 2, :]), preferred_element_type=f32)
        for r in range(t, RT):
            os_[r] = os_[r] + ot[(r - t) * 128:(r - t + 1) * 128]
    for r in range(RT):
        lo = base + r * 128
        ctx_h[lo // 2:(lo + 128) // 2, :] = _pk((os_[r] * _recip(ls[r])).astype(bf16))


def _b_head(b, xb, ckv, wd, q_s, k_s, v_s, ctx):
    h = (b % (HB // 2)) * 2 + b // (HB // 2)
    blk = pl.ds(b * PK, DC // 2)
    wq = _upk(jnp.concatenate([wd[0, blk, :], wd[1, blk, :]], axis=0))
    q = jnp.dot(xb[...], wq, preferred_element_type=f32) * SCALE_B
    q_s[...] = _pk(q.astype(bf16))
    wkv = _upk(jnp.concatenate([wd[2, blk, :], wd[3, blk, :]], axis=1))
    kv = jnp.dot(ckv[...], wkv, preferred_element_type=f32)
    k_s[...] = _pk(kv[:, :DB].astype(bf16))
    v_s[...] = _pk(kv[:, DB:].astype(bf16))
    ctx_h = ctx.at[h]
    order = list(range(NQ))[::-1]
    nx = _b_qk(order[0], q_s, k_s)
    for n, i in enumerate(order):
        cu = nx
        if n + 1 < NQ:
            nx = _b_qk(order[n + 1], q_s, k_s)
        _b_softmax_pv(i, cu[0], cu[1], v_s, ctx_h)


XC = 256
WCH = (4, 2, 2)
SEM_W = (0, 4, 6)
SEM_WOA, SEM_CKV, SEM_XB, SEM_WOB, SEM_XA = 8, 9, 10, 11, 12
SEM_WU = SEM_XA + S // XC
NSEM_IN = SEM_WU + NU


def _kernel(xa_hbm, wqkv_hbm, woa_hbm, xb_hbm, ckv_hbm, wq_hbm, wuk_hbm, wuv_hbm, wob_hbm,
            out_hbm,
            xa, wqkv, woa, wt, wop, q0, k0, v0, q1, k1, v1, ob0, ob1, stage,
            xb, ckv, wraw, wob, wd, q_s, k_s, v_s, ctx,
            zero_s, sem_in, sem_a, sem_b):
    def in_copy(idx, src, dst):
        return pltpu.make_async_copy(src, dst, sem_in.at[idx])

    def rows(j, n):
        return pl.ds(j * n if isinstance(j, int) else pl.multiple_of(j * n, n), n)

    def c_w(t, c):
        r = rows(c, DM // WCH[t])
        cols = slice(t * DM, (t + 1) * DM)
        return in_copy(SEM_W[t] + c, wqkv_hbm.at[r, cols], wqkv.at[r, cols])

    def c_xa(j):
        return in_copy(SEM_XA + j, xa_hbm.at[rows(j, XC)], xa.at[rows(j, XC)])

    c_woa = in_copy(SEM_WOA, woa_hbm, woa)

    def c_wu_start(u):
        if u < 8:
            src = wq_hbm.at[rows(u, 128)]
        elif u < 12:
            src = wuk_hbm.at[rows(u - 8, 128)]
        else:
            src = wuv_hbm.at[rows(u - 12, 128)]
        in_copy(SEM_WU + u, src, wraw.at[rows(u, 128)]).start()

    def c_wu_wait(u):
        dst = wraw.at[rows(u, 128)]
        in_copy(SEM_WU + u, dst, dst).wait()

    c_ckv = in_copy(SEM_CKV, ckv_hbm, ckv)
    c_xb = in_copy(SEM_XB, xb_hbm, xb)
    c_wob = in_copy(SEM_WOB, wob_hbm, wob)

    def a_out_copy(i):
        return pltpu.make_async_copy(stage.at[rows(i, TA), :],
                                     out_hbm.at[rows(i, TA), 0:DM], sem_a.at[i])

    def b_out_copy(i, half):
        cols = slice(half * (DM // 2), (half + 1) * (DM // 2))
        ocols = slice(DM + half * (DM // 2), DM + (half + 1) * (DM // 2))
        return pltpu.make_async_copy(stage.at[rows(i, TO), cols],
                                     out_hbm.at[rows(i, TO), ocols], sem_b.at[2 * i + half])

    for c in range(WCH[0]):
        c_w(0, c).start()
    c_xa(0).start()
    for t in (1, 2):
        for c in range(WCH[t]):
            c_w(t, c).start()
    c_woa.start()
    for j in range(S // XC - 1):
        c_xa(j + 1).start()
        if j > 0:
            c_wu_start(2 * j - 1)
        c_wu_start(2 * j)
    for u in range(2 * (S // XC - 2) + 1, NU):
        c_wu_start(u)
    for c in (c_ckv, c_xb, c_wob):
        c.start()
    zero_s[0] = jnp.uint32(0)

    bufs = [(q0, k0, v0), (q1, k1, v1)]
    obuf = [ob0, ob1]
    k0[:, 0:HALO, :] = jnp.zeros((8, HALO, 128), f32)
    v0[:, 0:HALO, :] = jnp.zeros((8, HALO, 128), f32)
    proj = functools.partial(_a_proj_third, xa, wt)
    for c in range(4):
        c_w(0, c).wait()
        _prep_wt(wqkv, 0, wt, range(2 * c, 2 * c + 2))
    c_xa(0).wait()
    proj(0, 0, bufs[0])

    def piece(blk, t, half):
        _a_proj_piece(xa, wt, blk * TA, t * (DM // PC) + half, bufs[blk])

    c_w(1, 0).wait()
    piece(1, 0, 0)
    _prep_wt(wqkv, 1, wt, range(0, 4))
    c_w(1, 1).wait()
    piece(1, 0, 1)
    _prep_wt(wqkv, 1, wt, range(4, 8))
    proj(0, 1, bufs[0])
    c_w(2, 0).wait()
    piece(1, 1, 0)
    _prep_wt(wqkv, 2, wt, range(0, 4))
    c_w(2, 1).wait()
    piece(1, 1, 1)
    _prep_wt(wqkv, 2, wt, range(4, 8))
    proj(0, 2, bufs[0])
    c_woa.wait()
    for t in (1, 2):
        _a_halo(bufs[0], bufs[1], t)
    _a_attn(bufs, obuf, 0, 0)
    proj(1, 2, bufs[1])
    _prep_wo(woa, wop)

    st = functools.partial(_a_stage, xa, wt, wop, stage, a_out_copy, bufs, obuf)

    def a_body(j, carry):
        c_xa(j + 1).wait()

        @pl.when(j > 0)
        def _():
            c_wu_wait(2 * j - 1)

        c_wu_wait(2 * j)
        zero = jnp.full((8, 128), zero_s[0], u32)
        z = _b_deint_unit(wraw, wd, jnp.maximum(2 * j - 1, 0), zero)
        _b_deint_unit(wraw, wd, 2 * j, zero, z)
        st(2 * j + 1, 1, True)
        st(2 * j + 2, 0, True)
        return carry

    jax.lax.fori_loop(0, (NA - 2) // 2, a_body, 0)

    for u in range(NU - 3, NU):
        c_wu_wait(u)
    zero = jnp.full((8, 128), zero_s[0], u32)

    def last_units():
        z = _b_deint_unit(wraw, wd, NU - 3, zero, None, 0)
        _b_deint_unit(wraw, wd, NU - 2, zero, z, 0)
        _b_deint_unit(wraw, wd, NU - 1, zero, None, 0)

    st(NA - 1, 1, False, side=[last_units])
    _a_out(wop, stage, a_out_copy, obuf, NA - 1, 1)
    c_ckv.wait()
    c_xb.wait()

    def b_body(h, carry):
        _b_head(h, xb, ckv, wd, q_s, k_s, v_s, ctx)
        return carry

    jax.lax.fori_loop(0, HB, b_body, 0)

    c_wob.wait()
    for i in range(NA):
        a_out_copy(i).wait()

    def o_body(i, carry):
        r2 = pl.multiple_of(i * (TO // 2), TO // 2)
        lhs = jnp.concatenate(
            [_upk(ctx[h, pl.ds(r2, TO // 2), :]) for h in range(HB)], axis=1)
        for half in range(2):
            cols = slice(half * (DM // 2), (half + 1) * (DM // 2))
            y = jnp.dot(lhs, wob[:, cols], preferred_element_type=f32)
            stage[pl.ds(pl.multiple_of(i * TO, TO), TO), cols] = y.astype(bf16)
            b_out_copy(i, half).start()
        return carry

    jax.lax.fori_loop(0, S // TO, o_body, 0)
    for i in range(S // TO):
        for half in range(2):
            b_out_copy(i, half).wait()


@jax.jit
def pallas_concat_heads__sliding_local_dilated__compressed_kv_cla__prompt_kernel(
    A_x: jax.Array,
    A_wqkv: jax.Array,
    A_wo: jax.Array,
    B_x: jax.Array,
    B_c_kv: jax.Array,
    B_w_q: jax.Array,
    B_w_uk: jax.Array,
    B_w_uv: jax.Array,
    B_w_o: jax.Array,
):
    V = pltpu.VMEM
    slab = lambda n: V((8, n, 128), f32)
    scratch = [
        V((S, DM), bf16),
        V((DM, 3 * DM), bf16),
        V((DM, DM), bf16),
        V((DM // 128, 3 * NW, 128), u32),
        V((DM // 128, NW, 128), u32),
        slab(TA), slab(TA + HALO), slab(TA + HALO),
        slab(TA), slab(TA + HALO), slab(TA + HALO),
        V((TA // 2, DM), u32), V((TA // 2, DM), u32),
        V((S, DM), bf16),
        V((S, DM), bf16),
        V((S, DC), bf16),
        V((DM + 2 * DC, HB, DB), bf16),
        V((HB * DB, DM), bf16),
        V((4, HB * PK, DB), u32),
        V((S // 2, DB), u32), V((S // 2, DB), u32), V((S // 2, DB), u32),
        V((HB, S // 2, DB), u32),
        pltpu.SMEM((1,), u32),
        pltpu.SemaphoreType.DMA((NSEM_IN,)),
        pltpu.SemaphoreType.DMA((NA,)),
        pltpu.SemaphoreType.DMA((2 * (S // TO),)),
    ]
    any_spec = pl.BlockSpec(memory_space=pl.ANY)
    out = pl.pallas_call(
        _kernel,
        out_shape=jax.ShapeDtypeStruct((S, 2 * DM), bf16),
        in_specs=[any_spec] * 9,
        out_specs=any_spec,
        scratch_shapes=scratch,
        compiler_params=pltpu.CompilerParams(vmem_limit_bytes=120 * 1024 * 1024,
                                             disable_bounds_checks=True),
    )(
        A_x.reshape(S, DM), A_wqkv, A_wo,
        B_x.reshape(S, DM), B_c_kv.reshape(S, DC), B_w_q, B_w_uk, B_w_uv,
        B_w_o.reshape(HB * DB, DM),
    )
    return out.reshape(1, S, 2 * DM)
```

```python
import functools
import math

import jax
import jax.numpy as jnp
import jax.experimental.pallas as pl
import jax.experimental.pallas.tpu as pltpu

bf16 = jnp.bfloat16
f32 = jnp.float32
u32 = jnp.uint32

NEG = -1e9
LOG2E = math.log2(math.e)
NT = (((1,), (1,)), ((), ()))

S = 2048
DM = 1024
HA, DH, WIN, DIL = 32, 32, 8, 2
TA = 128
NA = S // TA
HALO = 16
RC = 64
PC = 512
SCALE_A = DH ** -0.5 * LOG2E
HB, DB, DC = 32, 128, 512
TQ = 256
NQ = S // TQ
RT = TQ // 128
SCALE_B = DB ** -0.5 * LOG2E
TO = 256


def _pk(x):
    return pltpu.bitcast(x, u32)


def _upk(x):
    return pltpu.bitcast(x, bf16)


def _tree(xs, op):
    xs = list(xs)
    while len(xs) > 1:
        xs = [op(xs[k], xs[k + 1]) if k + 1 < len(xs) else xs[k] for k in range(0, len(xs), 2)]
    return xs[0]


def _dot_nt(a, b):
    return jax.lax.dot_general(a, b, NT, preferred_element_type=f32)


def _recip(l):
    return pl.reciprocal(l, approx=False, full_range=False)


PW = HA // 2 + 1
NW = DH * PW


def _repack_heads(u, dst, base):
    for hp in range(HA // 2):
        a = u[(2 * hp) * 16:(2 * hp + 1) * 16]
        b = u[(2 * hp + 1) * 16:(2 * hp + 2) * 16]
        lo = (a & u32(0xFFFF)) | (b << 16)
        hi = (a >> 16) | (b & u32(0xFFFF0000))
        for k, v in enumerate((lo[0:8], lo[8:16], hi[0:8], hi[8:16])):
            dst[pl.ds(base + k * 8 * PW + hp, 8, stride=PW), :] = v


def _load_slots(src, base, s0, s1):
    return jnp.concatenate([src[base + d * PW:base + d * PW + 16, :] for d in range(s0, s1)], axis=0)


def _prep_wt(w_ref, t, wt_ref, mcs=range(DM // 128)):
    for mc in mcs:
        blk = w_ref[mc * 128:(mc + 1) * 128, t * DM:(t + 1) * DM]
        _repack_heads(_pk(blk.T), wt_ref.at[mc], t * NW)


def _prep_wo(wo_ref, wop_ref):
    for nc in range(DM // 128):
        _repack_heads(_pk(wo_ref[:, nc * 128:(nc + 1) * 128]), wop_ref.at[nc], 0)


def _a_proj_piece(x_ref, wt_ref, r0, n, nxt):
    x = x_ref[pl.ds(r0, TA), :]
    t, s0 = (n * PC) // DM, ((n * PC) % DM) // HA
    w = jnp.concatenate([_load_slots(wt_ref.at[mc], t * NW, s0, s0 + PC // HA)
                         for mc in range(DM // 128)], axis=1)
    y = _dot_nt(x, _upk(w))
    for j in range(PC // 128):
        col = n * PC + j * 128
        t, g = col // DM, (col % DM) // 128
        blk = y[:, j * 128:(j + 1) * 128]
        if t == 0:
            nxt[0][g, :, :] = blk * SCALE_A
        else:
            nxt[t][g, HALO:HALO + TA, :] = blk


def _a_attn_chunk(bufs, r0, c, o_ref):
    qv, kv, vv = bufs
    a = c * RC
    pos = r0 + a + jax.lax.broadcasted_iota(jnp.int32, (RC, 128), 0)
    q = [qv[g, a:a + RC, :] for g in range(8)]
    s = []
    for w in range(WIN):
        o = HALO + a - DIL * w
        acc = q[0] * kv[0, o:o + RC, :]
        for g in range(1, 8):
            acc = acc + q[g] * kv[g, o:o + RC, :]
        acc = acc + pltpu.roll(acc, 64, 1)
        acc = acc + pltpu.roll(acc, 32, 1)
        if w > 0:
            acc = jnp.where(pos >= DIL * w, acc, NEG)
        s.append(acc)
    m = s[0]
    for w in range(1, WIN):
        m = jnp.maximum(m, s[w])
    e = [jnp.exp2(s[w] - m) for w in range(WIN)]
    l = e[0]
    for w in range(1, WIN):
        l = l + e[w]
    inv = _recip(l)
    cols = []
    for g in range(8):
        acc = e[0] * vv[g, HALO + a:HALO + a + RC, :]
        for w in range(1, WIN):
            o = HALO + a - DIL * w
            acc = acc + e[w] * vv[g, o:o + RC, :]
        cols.append(acc * inv)
    o_ref[a // 2:(a + RC) // 2, :] = _pk(jnp.concatenate(cols, axis=1).astype(bf16))


def _a_out_piece(o_ref, wop_ref, stage_ref, r0, n):
    w = jnp.concatenate([_load_slots(wop_ref.at[nc], 0, 0, DH)
                         for nc in range(n * PC // 128, (n + 1) * PC // 128)], axis=1)
    y = jnp.dot(_upk(o_ref[...]), _upk(w), preferred_element_type=f32)
    stage_ref[pl.ds(r0, TA), n * PC:(n + 1) * PC] = y.astype(bf16)


def _a_halo(cur, nxt, t):
    nxt[t][:, 0:HALO, :] = cur[t][:, TA:TA + HALO, :]


def _a_proj_third(x_ref, wt_ref, blk, t, dst):
    rn = blk * TA
    if not isinstance(rn, int):
        rn = pl.multiple_of(rn, TA)
    for n in range(t * DM // PC, (t + 1) * DM // PC):
        _a_proj_piece(x_ref, wt_ref, rn, n, dst)


def _a_attn(bufs, obuf, i, par):
    for c in range(TA // RC):
        _a_attn_chunk(bufs[par], i * TA, c, obuf[par])


def _a_out(wop_ref, stage_ref, out_copy, obuf, i, par):
    rp = i * TA
    if not isinstance(rp, int):
        rp = pl.multiple_of(rp, TA)
    for n in range(DM // PC):
        _a_out_piece(obuf[par], wop_ref, stage_ref, rp, n)
    out_copy(i).start()


def _a_stage(x_ref, wt_ref, wop_ref, stage_ref, out_copy, bufs, obuf,
             i, par, do_proj, side=()):
    if do_proj:
        for t in (1, 2):
            _a_halo(bufs[par], bufs[1 - par], t)
    _a_attn(bufs, obuf, i, par)
    mm = []
    if do_proj:
        rn = (i + 1) * TA
        if not isinstance(rn, int):
            rn = pl.multiple_of(rn, TA)
        mm += [functools.partial(_a_proj_piece, x_ref, wt_ref, rn, n, bufs[1 - par])
               for n in range(3 * DM // PC)]
    rp = (i - 1) * TA
    if not isinstance(rp, int):
        rp = pl.multiple_of(rp, TA)
    mm += [functools.partial(_a_out_piece, obuf[1 - par], wop_ref, stage_ref, rp, n)
           for n in range(DM // PC)]
    for f in side:
        f()
    for f in mm:
        f()
    out_copy(i - 1).start()


PK = DC // 2 + 1
NU = 16


def _b_deint(raw, dst, pitch, r0, p0, zero=None, z=None, delay=None):
    span = (HB - 1) * pitch + 64
    view = dst.at[pl.ds(p0, span), :]
    src = raw.at[pl.ds(r0, 128)]
    for p in range(64):
        x = pltpu.bitcast(src[2 * p:2 * p + 2], u32)
        a, b = x[0], x[1]
        if z is not None:
            a = a | jnp.concatenate([z, z], axis=0)
        lo = (a & u32(0xFFFF)) | (b << 16)
        hi = (a >> 16) | (b & u32(0xFFFF0000))
        for c, v in ((0, lo), (1, hi)):
            for half in range(2):
                blk = c * (HB // 2) + half * 8
                view[pl.ds(blk * pitch + p, 8, stride=pitch), :] = v[half * 8:(half + 1) * 8, :]
        if zero is not None:
            t = lo | hi
            z = (t[0:8] | t[8:16]) & zero
            delay = DELAY_EVERY if delay is None else delay
            if delay and p % delay == delay - 1:
                z = pltpu.roll(z, 1, 1)
    return z


DELAY_EVERY = 3


def _mult(x, n):
    return x if isinstance(x, int) else pl.multiple_of(x, n)


def _b_deint_unit(wraw, wd, u, zero=None, z=None, delay=None):
    return _b_deint(wraw, wd.at[u // 4], PK, _mult(u * 128, 128), _mult((u % 4) * 64, 64),
                    zero, z, delay)


def _b_qk(i, q_s, k_s):
    base = i * TQ
    q = _upk(q_s[base // 2:(base + TQ) // 2, :])
    s0 = _dot_nt(q, _upk(k_s[0:(base + 128) // 2, :]))
    sd = [_dot_nt(q[t * 128:], _upk(k_s[(base + t * 128) // 2:(base + (t + 1) * 128) // 2, :]))
          for t in range(1, RT)]
    return s0, sd


NCHAIN = 6


def _b_softmax_pv(i, s0, sd, v_s, ctx_h, zero, chain):
    base = i * TQ
    row = jax.lax.broadcasted_iota(jnp.int32, (128, 128), 0)
    col = jax.lax.broadcasted_iota(jnp.int32, (128, 128), 1)
    tri = col <= row
    ps, ls = [], []
    for r in range(RT):
        parts = [s0[r * 128:(r + 1) * 128]]
        parts += [sd[t - 1][(r - t) * 128:(r - t + 1) * 128] for t in range(1, r + 1)]
        sr = jnp.concatenate(parts, axis=1) if len(parts) > 1 else parts[0]
        lr = base + (r + 1) * 128
        dg = jnp.where(tri, sr[:, lr - 128:], NEG)
        sr = jnp.concatenate([sr[:, :lr - 128], dg], axis=1) if lr > 128 else dg
        m = jnp.max(sr, axis=1, keepdims=True)
        p = jnp.exp2(sr - m)
        sums = []
        for g in range(128 // 8):
            xs = [p[g * 8:(g + 1) * 8, j * 128:(j + 1) * 128] for j in range(lr // 128)]
            acc = xs[0]
            c = chain[0] % NCHAIN
            chain[0] += 1
            if chain[1][c] is not None:
                acc = pltpu.bitcast(pltpu.bitcast(acc, u32) | chain[1][c], f32)
            for y in xs[1:]:
                acc = acc + y
            chain[1][c] = pltpu.bitcast(acc, u32) & zero
            sums.append(acc)
        ls.append(jnp.sum(jnp.concatenate(sums, axis=0), axis=1, keepdims=True))
        ps.append(p)
    p0 = jnp.concatenate([p[:, :base + 128] for p in ps], axis=0)
    o = jnp.dot(p0.astype(bf16), _upk(v_s[0:(base + 128) // 2, :]), preferred_element_type=f32)
    os_ = [o[r * 128:(r + 1) * 128] for r in range(RT)]
    for t in range(1, RT):
        lo, hi = base + t * 128, base + (t + 1) * 128
        pt = [ps[r][:, lo:hi] for r in range(t, RT)]
        pt = jnp.concatenate(pt, axis=0) if len(pt) > 1 else pt[0]
        ot = jnp.dot(pt.astype(bf16), _upk(v_s[lo // 2:hi // 2, :]), preferred_element_type=f32)
        for r in range(t, RT):
            os_[r] = os_[r] + ot[(r - t) * 128:(r - t + 1) * 128]
    for r in range(RT):
        lo = base + r * 128
        ctx_h[lo // 2:(lo + 128) // 2, :] = _pk((os_[r] * _recip(ls[r])).astype(bf16))


def _b_head(b, xb, ckv, wd, q_s, k_s, v_s, ctx, zero):
    h = (b % (HB // 2)) * 2 + b // (HB // 2)
    blk = pl.ds(b * PK, DC // 2)
    wq = _upk(jnp.concatenate([wd[0, blk, :], wd[1, blk, :]], axis=0))
    q = jnp.dot(xb[...], wq, preferred_element_type=f32) * SCALE_B
    q_s[...] = _pk(q.astype(bf16))
    wkv = _upk(jnp.concatenate([wd[2, blk, :], wd[3, blk, :]], axis=1))
    kv = jnp.dot(ckv[...], wkv, preferred_element_type=f32)
    k_s[...] = _pk(kv[:, :DB].astype(bf16))
    v_s[...] = _pk(kv[:, DB:].astype(bf16))
    ctx_h = ctx.at[h]
    order = list(range(NQ))[::-1]
    chain = [0, [None] * NCHAIN]
    nx = _b_qk(order[0], q_s, k_s)
    for n, i in enumerate(order):
        cu = nx
        if n + 1 < NQ:
            nx = _b_qk(order[n + 1], q_s, k_s)
        _b_softmax_pv(i, cu[0], cu[1], v_s, ctx_h, zero, chain)


XC = 256
WCH = (4, 2, 2)
SEM_W = (0, 4, 6)
SEM_WOA, SEM_CKV, SEM_XB, SEM_WOB, SEM_XA = 8, 9, 10, 11, 12
SEM_WU = SEM_XA + S // XC
NSEM_IN = SEM_WU + NU


def _kernel(xa_hbm, wqkv_hbm, woa_hbm, xb_hbm, ckv_hbm, wq_hbm, wuk_hbm, wuv_hbm, wob_hbm,
            out_hbm,
            xa, wqkv, woa, wt, wop, q0, k0, v0, q1, k1, v1, ob0, ob1, stage,
            xb, ckv, wraw, wob, wd, q_s, k_s, v_s, ctx,
            zero_s, sem_in, sem_a, sem_b):
    def in_copy(idx, src, dst):
        return pltpu.make_async_copy(src, dst, sem_in.at[idx])

    def rows(j, n):
        return pl.ds(j * n if isinstance(j, int) else pl.multiple_of(j * n, n), n)

    def c_w(t, c):
        r = rows(c, DM // WCH[t])
        cols = slice(t * DM, (t + 1) * DM)
        return in_copy(SEM_W[t] + c, wqkv_hbm.at[r, cols], wqkv.at[r, cols])

    def c_xa(j):
        return in_copy(SEM_XA + j, xa_hbm.at[rows(j, XC)], xa.at[rows(j, XC)])

    c_woa = in_copy(SEM_WOA, woa_hbm, woa)

    def c_wu_start(u):
        if u < 8:
            src = wq_hbm.at[rows(u, 128)]
        elif u < 12:
            src = wuk_hbm.at[rows(u - 8, 128)]
        else:
            src = wuv_hbm.at[rows(u - 12, 128)]
        in_copy(SEM_WU + u, src, wraw.at[rows(u, 128)]).start()

    def c_wu_wait(u):
        dst = wraw.at[rows(u, 128)]
        in_copy(SEM_WU + u, dst, dst).wait()

    c_ckv = in_copy(SEM_CKV, ckv_hbm, ckv)
    c_xb = in_copy(SEM_XB, xb_hbm, xb)
    c_wob = in_copy(SEM_WOB, wob_hbm, wob)

    def a_out_copy(i):
        return pltpu.make_async_copy(stage.at[rows(i, TA), :],
                                     out_hbm.at[rows(i, TA), 0:DM], sem_a.at[i])

    def b_out_copy(i, half):
        cols = slice(half * (DM // 2), (half + 1) * (DM // 2))
        ocols = slice(DM + half * (DM // 2), DM + (half + 1) * (DM // 2))
        return pltpu.make_async_copy(stage.at[rows(i, TO), cols],
                                     out_hbm.at[rows(i, TO), ocols], sem_b.at[2 * i + half])

    for c in range(WCH[0]):
        c_w(0, c).start()
    c_xa(0).start()
    for t in (1, 2):
        for c in range(WCH[t]):
            c_w(t, c).start()
    c_woa.start()
    for j in range(S // XC - 1):
        c_xa(j + 1).start()
        if j > 0:
            c_wu_start(2 * j - 1)
        c_wu_start(2 * j)
    for u in range(2 * (S // XC - 2) + 1, NU):
        c_wu_start(u)
    for c in (c_ckv, c_xb, c_wob):
        c.start()
    zero_s[0] = jnp.uint32(0)

    bufs = [(q0, k0, v0), (q1, k1, v1)]
    obuf = [ob0, ob1]
    k0[:, 0:HALO, :] = jnp.zeros((8, HALO, 128), f32)
    v0[:, 0:HALO, :] = jnp.zeros((8, HALO, 128), f32)
    proj = functools.partial(_a_proj_third, xa, wt)
    for c in range(4):
        c_w(0, c).wait()
        _prep_wt(wqkv, 0, wt, range(2 * c, 2 * c + 2))
    c_xa(0).wait()
    proj(0, 0, bufs[0])

    def piece(blk, t, half):
        _a_proj_piece(xa, wt, blk * TA, t * (DM // PC) + half, bufs[blk])

    c_w(1, 0).wait()
    piece(1, 0, 0)
    _prep_wt(wqkv, 1, wt, range(0, 4))
    c_w(1, 1).wait()
    piece(1, 0, 1)
    _prep_wt(wqkv, 1, wt, range(4, 8))
    proj(0, 1, bufs[0])
    c_w(2, 0).wait()
    piece(1, 1, 0)
    _prep_wt(wqkv, 2, wt, range(0, 4))
    c_w(2, 1).wait()
    piece(1, 1, 1)
    _prep_wt(wqkv, 2, wt, range(4, 8))
    proj(0, 2, bufs[0])
    c_woa.wait()
    for t in (1, 2):
        _a_halo(bufs[0], bufs[1], t)
    _a_attn(bufs, obuf, 0, 0)
    proj(1, 2, bufs[1])
    _prep_wo(woa, wop)

    st = functools.partial(_a_stage, xa, wt, wop, stage, a_out_copy, bufs, obuf)

    def a_body(j, carry):
        c_xa(j + 1).wait()

        @pl.when(j > 0)
        def _():
            c_wu_wait(2 * j - 1)

        c_wu_wait(2 * j)
        zero = jnp.full((8, 128), zero_s[0], u32)
        z = _b_deint_unit(wraw, wd, jnp.maximum(2 * j - 1, 0), zero)
        _b_deint_unit(wraw, wd, 2 * j, zero, z)
        st(2 * j + 1, 1, True)
        st(2 * j + 2, 0, True)
        return carry

    jax.lax.fori_loop(0, (NA - 2) // 2, a_body, 0)

    for u in range(NU - 3, NU):
        c_wu_wait(u)
    zero = jnp.full((8, 128), zero_s[0], u32)

    def last_units():
        z = _b_deint_unit(wraw, wd, NU - 3, zero, None, 0)
        _b_deint_unit(wraw, wd, NU - 2, zero, z, 0)
        _b_deint_unit(wraw, wd, NU - 1, zero, None, 0)

    st(NA - 1, 1, False, side=[last_units])
    _a_out(wop, stage, a_out_copy, obuf, NA - 1, 1)
    c_ckv.wait()
    c_xb.wait()

    def b_body(h, carry):
        zero = jnp.full((8, 128), zero_s[0], u32)
        _b_head(h, xb, ckv, wd, q_s, k_s, v_s, ctx, zero)
        return carry

    jax.lax.fori_loop(0, HB, b_body, 0)

    c_wob.wait()
    for i in range(NA):
        a_out_copy(i).wait()

    def o_body(i, carry):
        r2 = pl.multiple_of(i * (TO // 2), TO // 2)
        lhs = jnp.concatenate(
            [_upk(ctx[h, pl.ds(r2, TO // 2), :]) for h in range(HB)], axis=1)
        for half in range(2):
            cols = slice(half * (DM // 2), (half + 1) * (DM // 2))
            y = jnp.dot(lhs, wob[:, cols], preferred_element_type=f32)
            stage[pl.ds(pl.multiple_of(i * TO, TO), TO), cols] = y.astype(bf16)
            b_out_copy(i, half).start()
        return carry

    jax.lax.fori_loop(0, S // TO, o_body, 0)
    for i in range(S // TO):
        for half in range(2):
            b_out_copy(i, half).wait()


@jax.jit
def pallas_concat_heads__sliding_local_dilated__compressed_kv_cla__prompt_kernel(
    A_x: jax.Array,
    A_wqkv: jax.Array,
    A_wo: jax.Array,
    B_x: jax.Array,
    B_c_kv: jax.Array,
    B_w_q: jax.Array,
    B_w_uk: jax.Array,
    B_w_uv: jax.Array,
    B_w_o: jax.Array,
):
    V = pltpu.VMEM
    slab = lambda n: V((8, n, 128), f32)
    scratch = [
        V((S, DM), bf16),
        V((DM, 3 * DM), bf16),
        V((DM, DM), bf16),
        V((DM // 128, 3 * NW, 128), u32),
        V((DM // 128, NW, 128), u32),
        slab(TA), slab(TA + HALO), slab(TA + HALO),
        slab(TA), slab(TA + HALO), slab(TA + HALO),
        V((TA // 2, DM), u32), V((TA // 2, DM), u32),
        V((S, DM), bf16),
        V((S, DM), bf16),
        V((S, DC), bf16),
        V((DM + 2 * DC, HB, DB), bf16),
        V((HB * DB, DM), bf16),
        V((4, HB * PK, DB), u32),
        V((S // 2, DB), u32), V((S // 2, DB), u32), V((S // 2, DB), u32),
        V((HB, S // 2, DB), u32),
        pltpu.SMEM((1,), u32),
        pltpu.SemaphoreType.DMA((NSEM_IN,)),
        pltpu.SemaphoreType.DMA((NA,)),
        pltpu.SemaphoreType.DMA((2 * (S // TO),)),
    ]
    any_spec = pl.BlockSpec(memory_space=pl.ANY)
    out = pl.pallas_call(
        _kernel,
        out_shape=jax.ShapeDtypeStruct((S, 2 * DM), bf16),
        in_specs=[any_spec] * 9,
        out_specs=any_spec,
        scratch_shapes=scratch,
        compiler_params=pltpu.CompilerParams(vmem_limit_bytes=120 * 1024 * 1024,
                                             disable_bounds_checks=True),
    )(
        A_x.reshape(S, DM), A_wqkv, A_wo,
        B_x.reshape(S, DM), B_c_kv.reshape(S, DC), B_w_q, B_w_uk, B_w_uv,
        B_w_o.reshape(HB * DB, DM),
    )
    return out.reshape(1, S, 2 * DM)
```

```python
import functools
import math

import jax
import jax.numpy as jnp
import jax.experimental.pallas as pl
import jax.experimental.pallas.tpu as pltpu

bf16 = jnp.bfloat16
f32 = jnp.float32
u32 = jnp.uint32

NEG = -1e9
LOG2E = math.log2(math.e)
NT = (((1,), (1,)), ((), ()))

S = 2048
DM = 1024
HA, DH, WIN, DIL = 32, 32, 8, 2
TA = 128
NA = S // TA
HALO = 16
RC = 64
PC = 512
SCALE_A = DH ** -0.5 * LOG2E
HB, DB, DC = 32, 128, 512
TQ = 256
NQ = S // TQ
RT = TQ // 128
SCALE_B = DB ** -0.5 * LOG2E
TO = 256


def _pk(x):
    return pltpu.bitcast(x, u32)


def _upk(x):
    return pltpu.bitcast(x, bf16)


def _tree(xs, op):
    xs = list(xs)
    while len(xs) > 1:
        xs = [op(xs[k], xs[k + 1]) if k + 1 < len(xs) else xs[k] for k in range(0, len(xs), 2)]
    return xs[0]


def _dot_nt(a, b):
    return jax.lax.dot_general(a, b, NT, preferred_element_type=f32)


def _recip(l):
    return pl.reciprocal(l, approx=False, full_range=False)


PW = HA // 2 + 1
NW = DH * PW


def _repack_heads(u, dst, base):
    for hp in range(HA // 2):
        a = u[(2 * hp) * 16:(2 * hp + 1) * 16]
        b = u[(2 * hp + 1) * 16:(2 * hp + 2) * 16]
        lo = (a & u32(0xFFFF)) | (b << 16)
        hi = (a >> 16) | (b & u32(0xFFFF0000))
        for k, v in enumerate((lo[0:8], lo[8:16], hi[0:8], hi[8:16])):
            dst[pl.ds(base + k * 8 * PW + hp, 8, stride=PW), :] = v


def _load_slots(src, base, s0, s1):
    return jnp.concatenate([src[base + d * PW:base + d * PW + 16, :] for d in range(s0, s1)], axis=0)


def _prep_wt(w_ref, t, wt_ref, mcs=range(DM // 128)):
    for mc in mcs:
        blk = w_ref[mc * 128:(mc + 1) * 128, t * DM:(t + 1) * DM]
        _repack_heads(_pk(blk.T), wt_ref.at[mc], t * NW)


def _prep_wo(wo_ref, wop_ref):
    for nc in range(DM // 128):
        _repack_heads(_pk(wo_ref[:, nc * 128:(nc + 1) * 128]), wop_ref.at[nc], 0)


def _a_proj_piece(x_ref, wt_ref, r0, n, nxt):
    x = x_ref[pl.ds(r0, TA), :]
    t, s0 = (n * PC) // DM, ((n * PC) % DM) // HA
    w = jnp.concatenate([_load_slots(wt_ref.at[mc], t * NW, s0, s0 + PC // HA)
                         for mc in range(DM // 128)], axis=1)
    y = _dot_nt(x, _upk(w))
    for j in range(PC // 128):
        col = n * PC + j * 128
        t, g = col // DM, (col % DM) // 128
        blk = y[:, j * 128:(j + 1) * 128]
        if t == 0:
            nxt[0][g, :, :] = blk * SCALE_A
        else:
            nxt[t][g, HALO:HALO + TA, :] = blk


def _a_attn_chunk(bufs, r0, c, o_ref):
    qv, kv, vv = bufs
    a = c * RC
    pos = r0 + a + jax.lax.broadcasted_iota(jnp.int32, (RC, 128), 0)
    q = [qv[g, a:a + RC, :] for g in range(8)]
    s = []
    for w in range(WIN):
        o = HALO + a - DIL * w
        acc = q[0] * kv[0, o:o + RC, :]
        for g in range(1, 8):
            acc = acc + q[g] * kv[g, o:o + RC, :]
        acc = acc + pltpu.roll(acc, 64, 1)
        acc = acc + pltpu.roll(acc, 32, 1)
        if w > 0:
            acc = jnp.where(pos >= DIL * w, acc, NEG)
        s.append(acc)
    m = s[0]
    for w in range(1, WIN):
        m = jnp.maximum(m, s[w])
    e = [jnp.exp2(s[w] - m) for w in range(WIN)]
    l = e[0]
    for w in range(1, WIN):
        l = l + e[w]
    inv = _recip(l)
    cols = []
    for g in range(8):
        acc = e[0] * vv[g, HALO + a:HALO + a + RC, :]
        for w in range(1, WIN):
            o = HALO + a - DIL * w
            acc = acc + e[w] * vv[g, o:o + RC, :]
        cols.append(acc * inv)
    o_ref[a // 2:(a + RC) // 2, :] = _pk(jnp.concatenate(cols, axis=1).astype(bf16))


def _a_out_piece(o_ref, wop_ref, stage_ref, r0, n):
    w = jnp.concatenate([_load_slots(wop_ref.at[nc], 0, 0, DH)
                         for nc in range(n * PC // 128, (n + 1) * PC // 128)], axis=1)
    y = jnp.dot(_upk(o_ref[...]), _upk(w), preferred_element_type=f32)
    stage_ref[pl.ds(r0, TA), n * PC:(n + 1) * PC] = y.astype(bf16)


def _a_halo(cur, nxt, t):
    nxt[t][:, 0:HALO, :] = cur[t][:, TA:TA + HALO, :]


def _a_proj_third(x_ref, wt_ref, blk, t, dst):
    rn = blk * TA
    if not isinstance(rn, int):
        rn = pl.multiple_of(rn, TA)
    for n in range(t * DM // PC, (t + 1) * DM // PC):
        _a_proj_piece(x_ref, wt_ref, rn, n, dst)


def _a_attn(bufs, obuf, i, par):
    for c in range(TA // RC):
        _a_attn_chunk(bufs[par], i * TA, c, obuf[par])


def _a_out(wop_ref, stage_ref, out_copy, obuf, i, par):
    rp = i * TA
    if not isinstance(rp, int):
        rp = pl.multiple_of(rp, TA)
    for n in range(DM // PC):
        _a_out_piece(obuf[par], wop_ref, stage_ref, rp, n)
    out_copy(i).start()


def _a_stage(x_ref, wt_ref, wop_ref, stage_ref, out_copy, bufs, obuf,
             i, par, do_proj, side=()):
    if do_proj:
        for t in (1, 2):
            _a_halo(bufs[par], bufs[1 - par], t)
    _a_attn(bufs, obuf, i, par)
    mm = []
    if do_proj:
        rn = (i + 1) * TA
        if not isinstance(rn, int):
            rn = pl.multiple_of(rn, TA)
        mm += [functools.partial(_a_proj_piece, x_ref, wt_ref, rn, n, bufs[1 - par])
               for n in range(3 * DM // PC)]
    rp = (i - 1) * TA
    if not isinstance(rp, int):
        rp = pl.multiple_of(rp, TA)
    mm += [functools.partial(_a_out_piece, obuf[1 - par], wop_ref, stage_ref, rp, n)
           for n in range(DM // PC)]
    for f in side:
        f()
    for f in mm:
        f()
    out_copy(i - 1).start()


PK = DC // 2 + 1
NU = 16


def _b_deint(raw, dst, pitch, r0, p0, zero=None, z=None, delay=None):
    span = (HB - 1) * pitch + 64
    view = dst.at[pl.ds(p0, span), :]
    src = raw.at[pl.ds(r0, 128)]
    for p in range(64):
        x = pltpu.bitcast(src[2 * p:2 * p + 2], u32)
        a, b = x[0], x[1]
        if z is not None:
            a = a | jnp.concatenate([z, z], axis=0)
        lo = (a & u32(0xFFFF)) | (b << 16)
        hi = (a >> 16) | (b & u32(0xFFFF0000))
        for c, v in ((0, lo), (1, hi)):
            for half in range(2):
                blk = c * (HB // 2) + half * 8
                view[pl.ds(blk * pitch + p, 8, stride=pitch), :] = v[half * 8:(half + 1) * 8, :]
        if zero is not None:
            t = lo | hi
            z = (t[0:8] | t[8:16]) & zero
            delay = DELAY_EVERY if delay is None else delay
            if delay and p % delay == delay - 1:
                z = pltpu.roll(z, 1, 1)
    return z


DELAY_EVERY = 3


def _mult(x, n):
    return x if isinstance(x, int) else pl.multiple_of(x, n)


def _b_deint_unit(wraw, wd, u, zero=None, z=None, delay=None):
    return _b_deint(wraw, wd.at[u // 4], PK, _mult(u * 128, 128), _mult((u % 4) * 64, 64),
                    zero, z, delay)


def _b_qk(i, q_s, k_s):
    base = i * TQ
    q = _upk(q_s[base // 2:(base + TQ) // 2, :])
    s0 = _dot_nt(q, _upk(k_s[0:(base + 128) // 2, :]))
    sd = [_dot_nt(q[t * 128:], _upk(k_s[(base + t * 128) // 2:(base + (t + 1) * 128) // 2, :]))
          for t in range(1, RT)]
    return s0, sd


NCHAIN = 6
FREE_BLOCKS = 4


def _b_softmax_pv(i, s0, sd, v_s, ctx_h, zero, chain):
    base = i * TQ
    row = jax.lax.broadcasted_iota(jnp.int32, (128, 128), 0)
    col = jax.lax.broadcasted_iota(jnp.int32, (128, 128), 1)
    tri = col <= row
    ps, ls = [], []
    for r in range(RT):
        parts = [s0[r * 128:(r + 1) * 128]]
        parts += [sd[t - 1][(r - t) * 128:(r - t + 1) * 128] for t in range(1, r + 1)]
        sr = jnp.concatenate(parts, axis=1) if len(parts) > 1 else parts[0]
        lr = base + (r + 1) * 128
        dg = jnp.where(tri, sr[:, lr - 128:], NEG)
        sr = jnp.concatenate([sr[:, :lr - 128], dg], axis=1) if lr > 128 else dg
        m = jnp.max(sr, axis=1, keepdims=True)
        p = jnp.exp2(sr - m)
        sums = []
        for g in range(128 // 8):
            xs = [p[g * 8:(g + 1) * 8, j * 128:(j + 1) * 128] for j in range(lr // 128)]
            acc = xs[0]
            c = chain[0] % NCHAIN
            chain[0] += 1
            if i < FREE_BLOCKS:
                sums.append(_tree(xs, jnp.add))
                continue
            if chain[1][c] is not None:
                acc = pltpu.bitcast(pltpu.bitcast(acc, u32) | chain[1][c], f32)
            for y in xs[1:]:
                acc = acc + y
            chain[1][c] = pltpu.bitcast(acc, u32) & zero
            sums.append(acc)
        ls.append(jnp.sum(jnp.concatenate(sums, axis=0), axis=1, keepdims=True))
        ps.append(p)
    p0 = jnp.concatenate([p[:, :base + 128] for p in ps], axis=0)
    o = jnp.dot(p0.astype(bf16), _upk(v_s[0:(base + 128) // 2, :]), preferred_element_type=f32)
    os_ = [o[r * 128:(r + 1) * 128] for r in range(RT)]
    for t in range(1, RT):
        lo, hi = base + t * 128, base + (t + 1) * 128
        pt = [ps[r][:, lo:hi] for r in range(t, RT)]
        pt = jnp.concatenate(pt, axis=0) if len(pt) > 1 else pt[0]
        ot = jnp.dot(pt.astype(bf16), _upk(v_s[lo // 2:hi // 2, :]), preferred_element_type=f32)
        for r in range(t, RT):
            os_[r] = os_[r] + ot[(r - t) * 128:(r - t + 1) * 128]
    for r in range(RT):
        lo = base + r * 128
        ctx_h[lo // 2:(lo + 128) // 2, :] = _pk((os_[r] * _recip(ls[r])).astype(bf16))


def _b_head(b, xb, ckv, wd, q_s, k_s, v_s, ctx, zero):
    h = (b % (HB // 2)) * 2 + b // (HB // 2)
    blk = pl.ds(b * PK, DC // 2)
    wq = _upk(jnp.concatenate([wd[0, blk, :], wd[1, blk, :]], axis=0))
    q = jnp.dot(xb[...], wq, preferred_element_type=f32) * SCALE_B
    q_s[...] = _pk(q.astype(bf16))
    wkv = _upk(jnp.concatenate([wd[2, blk, :], wd[3, blk, :]], axis=1))
    kv = jnp.dot(ckv[...], wkv, preferred_element_type=f32)
    k_s[...] = _pk(kv[:, :DB].astype(bf16))
    v_s[...] = _pk(kv[:, DB:].astype(bf16))
    ctx_h = ctx.at[h]
    order = list(range(NQ))[::-1]
    chain = [0, [None] * NCHAIN]
    nx = _b_qk(order[0], q_s, k_s)
    for n, i in enumerate(order):
        cu = nx
        if n + 1 < NQ:
            nx = _b_qk(order[n + 1], q_s, k_s)
        _b_softmax_pv(i, cu[0], cu[1], v_s, ctx_h, zero, chain)


XC = 256
WCH = (4, 2, 2)
SEM_W = (0, 4, 6)
SEM_WOA, SEM_CKV, SEM_XB, SEM_WOB, SEM_XA = 8, 9, 10, 11, 12
SEM_WU = SEM_XA + S // XC
NSEM_IN = SEM_WU + NU


def _kernel(xa_hbm, wqkv_hbm, woa_hbm, xb_hbm, ckv_hbm, wq_hbm, wuk_hbm, wuv_hbm, wob_hbm,
            out_hbm,
            xa, wqkv, woa, wt, wop, q0, k0, v0, q1, k1, v1, ob0, ob1, stage,
            xb, ckv, wraw, wob, wd, q_s, k_s, v_s, ctx,
            zero_s, sem_in, sem_a, sem_b):
    def in_copy(idx, src, dst):
        return pltpu.make_async_copy(src, dst, sem_in.at[idx])

    def rows(j, n):
        return pl.ds(j * n if isinstance(j, int) else pl.multiple_of(j * n, n), n)

    def c_w(t, c):
        r = rows(c, DM // WCH[t])
        cols = slice(t * DM, (t + 1) * DM)
        return in_copy(SEM_W[t] + c, wqkv_hbm.at[r, cols], wqkv.at[r, cols])

    def c_xa(j):
        return in_copy(SEM_XA + j, xa_hbm.at[rows(j, XC)], xa.at[rows(j, XC)])

    c_woa = in_copy(SEM_WOA, woa_hbm, woa)

    def c_wu_start(u):
        if u < 8:
            src = wq_hbm.at[rows(u, 128)]
        elif u < 12:
            src = wuk_hbm.at[rows(u - 8, 128)]
        else:
            src = wuv_hbm.at[rows(u - 12, 128)]
        in_copy(SEM_WU + u, src, wraw.at[rows(u, 128)]).start()

    def c_wu_wait(u):
        dst = wraw.at[rows(u, 128)]
        in_copy(SEM_WU + u, dst, dst).wait()

    c_ckv = in_copy(SEM_CKV, ckv_hbm, ckv)
    c_xb = in_copy(SEM_XB, xb_hbm, xb)
    c_wob = in_copy(SEM_WOB, wob_hbm, wob)

    def a_out_copy(i):
        return pltpu.make_async_copy(stage.at[rows(i, TA), :],
                                     out_hbm.at[rows(i, TA), 0:DM], sem_a.at[i])

    def b_out_copy(i, half):
        cols = slice(half * (DM // 2), (half + 1) * (DM // 2))
        ocols = slice(DM + half * (DM // 2), DM + (half + 1) * (DM // 2))
        return pltpu.make_async_copy(stage.at[rows(i, TO), cols],
                                     out_hbm.at[rows(i, TO), ocols], sem_b.at[2 * i + half])

    for c in range(WCH[0]):
        c_w(0, c).start()
    c_xa(0).start()
    for t in (1, 2):
        for c in range(WCH[t]):
            c_w(t, c).start()
    c_woa.start()
    for j in range(S // XC - 1):
        c_xa(j + 1).start()
        if j > 0:
            c_wu_start(2 * j - 1)
        c_wu_start(2 * j)
    for u in range(2 * (S // XC - 2) + 1, NU):
        c_wu_start(u)
    for c in (c_ckv, c_xb, c_wob):
        c.start()
    zero_s[0] = jnp.uint32(0)

    bufs = [(q0, k0, v0), (q1, k1, v1)]
    obuf = [ob0, ob1]
    k0[:, 0:HALO, :] = jnp.zeros((8, HALO, 128), f32)
    v0[:, 0:HALO, :] = jnp.zeros((8, HALO, 128), f32)
    proj = functools.partial(_a_proj_third, xa, wt)
    for c in range(4):
        c_w(0, c).wait()
        _prep_wt(wqkv, 0, wt, range(2 * c, 2 * c + 2))
    c_xa(0).wait()
    proj(0, 0, bufs[0])

    def piece(blk, t, half):
        _a_proj_piece(xa, wt, blk * TA, t * (DM // PC) + half, bufs[blk])

    c_w(1, 0).wait()
    piece(1, 0, 0)
    _prep_wt(wqkv, 1, wt, range(0, 4))
    c_w(1, 1).wait()
    piece(1, 0, 1)
    _prep_wt(wqkv, 1, wt, range(4, 8))
    proj(0, 1, bufs[0])
    c_w(2, 0).wait()
    piece(1, 1, 0)
    _prep_wt(wqkv, 2, wt, range(0, 4))
    c_w(2, 1).wait()
    piece(1, 1, 1)
    _prep_wt(wqkv, 2, wt, range(4, 8))
    proj(0, 2, bufs[0])
    for t in (1, 2):
        _a_halo(bufs[0], bufs[1], t)
    _a_attn(bufs, obuf, 0, 0)
    proj(1, 2, bufs[1])
    c_woa.wait()
    _prep_wo(woa, wop)

    st = functools.partial(_a_stage, xa, wt, wop, stage, a_out_copy, bufs, obuf)

    def a_body(j, carry):
        c_xa(j + 1).wait()

        @pl.when(j > 0)
        def _():
            c_wu_wait(2 * j - 1)

        c_wu_wait(2 * j)
        zero = jnp.full((8, 128), zero_s[0], u32)
        z = _b_deint_unit(wraw, wd, jnp.maximum(2 * j - 1, 0), zero)
        _b_deint_unit(wraw, wd, 2 * j, zero, z)
        st(2 * j + 1, 1, True)
        st(2 * j + 2, 0, True)
        return carry

    jax.lax.fori_loop(0, (NA - 2) // 2, a_body, 0)

    for u in range(NU - 3, NU):
        c_wu_wait(u)
    zero = jnp.full((8, 128), zero_s[0], u32)

    def last_units():
        z = _b_deint_unit(wraw, wd, NU - 3, zero, None, 0)
        _b_deint_unit(wraw, wd, NU - 2, zero, z, 0)
        _b_deint_unit(wraw, wd, NU - 1, zero, None, 0)

    st(NA - 1, 1, False, side=[last_units])
    _a_out(wop, stage, a_out_copy, obuf, NA - 1, 1)
    c_ckv.wait()
    c_xb.wait()

    def b_body(h, carry):
        zero = jnp.full((8, 128), zero_s[0], u32)
        _b_head(h, xb, ckv, wd, q_s, k_s, v_s, ctx, zero)
        return carry

    jax.lax.fori_loop(0, HB, b_body, 0)

    c_wob.wait()
    for i in range(NA):
        a_out_copy(i).wait()

    def o_body(i, carry):
        r2 = pl.multiple_of(i * (TO // 2), TO // 2)
        lhs = jnp.concatenate(
            [_upk(ctx[h, pl.ds(r2, TO // 2), :]) for h in range(HB)], axis=1)
        for half in range(2):
            cols = slice(half * (DM // 2), (half + 1) * (DM // 2))
            y = jnp.dot(lhs, wob[:, cols], preferred_element_type=f32)
            stage[pl.ds(pl.multiple_of(i * TO, TO), TO), cols] = y.astype(bf16)
            b_out_copy(i, half).start()
        return carry

    jax.lax.fori_loop(0, S // TO, o_body, 0)
    for i in range(S // TO):
        for half in range(2):
            b_out_copy(i, half).wait()


@jax.jit
def pallas_concat_heads__sliding_local_dilated__compressed_kv_cla__prompt_kernel(
    A_x: jax.Array,
    A_wqkv: jax.Array,
    A_wo: jax.Array,
    B_x: jax.Array,
    B_c_kv: jax.Array,
    B_w_q: jax.Array,
    B_w_uk: jax.Array,
    B_w_uv: jax.Array,
    B_w_o: jax.Array,
):
    V = pltpu.VMEM
    slab = lambda n: V((8, n, 128), f32)
    scratch = [
        V((S, DM), bf16),
        V((DM, 3 * DM), bf16),
        V((DM, DM), bf16),
        V((DM // 128, 3 * NW, 128), u32),
        V((DM // 128, NW, 128), u32),
        slab(TA), slab(TA + HALO), slab(TA + HALO),
        slab(TA), slab(TA + HALO), slab(TA + HALO),
        V((TA // 2, DM), u32), V((TA // 2, DM), u32),
        V((S, DM), bf16),
        V((S, DM), bf16),
        V((S, DC), bf16),
        V((DM + 2 * DC, HB, DB), bf16),
        V((HB * DB, DM), bf16),
        V((4, HB * PK, DB), u32),
        V((S // 2, DB), u32), V((S // 2, DB), u32), V((S // 2, DB), u32),
        V((HB, S // 2, DB), u32),
        pltpu.SMEM((1,), u32),
        pltpu.SemaphoreType.DMA((NSEM_IN,)),
        pltpu.SemaphoreType.DMA((NA,)),
        pltpu.SemaphoreType.DMA((2 * (S // TO),)),
    ]
    any_spec = pl.BlockSpec(memory_space=pl.ANY)
    out = pl.pallas_call(
        _kernel,
        out_shape=jax.ShapeDtypeStruct((S, 2 * DM), bf16),
        in_specs=[any_spec] * 9,
        out_specs=any_spec,
        scratch_shapes=scratch,
        compiler_params=pltpu.CompilerParams(vmem_limit_bytes=120 * 1024 * 1024,
                                             disable_bounds_checks=True),
    )(
        A_x.reshape(S, DM), A_wqkv, A_wo,
        B_x.reshape(S, DM), B_c_kv.reshape(S, DC), B_w_q, B_w_uk, B_w_uv,
        B_w_o.reshape(HB * DB, DM),
    )
    return out.reshape(1, S, 2 * DM)
```
